```python
import jax
import jax.numpy as jnp

def _softmax(x, axis=-1):
    return jax.nn.softmax(x, axis=axis)

def _gelu(x):
    return jax.nn.gelu(x, approximate=True)

def _silu(x):
    return jax.nn.silu(x)

def _sigmoid(x):
    return jax.nn.sigmoid(x)

def _layernorm(x, axis=-1, eps=1e-05):
    m = jnp.mean(x, axis=axis, keepdims=True)
    v = jnp.var(x, axis=axis, keepdims=True)
    return (x - m) / jnp.sqrt(v + eps)

def _scatter_add(tgt, idx, src, axis=0):
    return tgt.at[idx].add(src)

def _segment_sum(src, seg, n):
    return jax.ops.segment_sum(src, seg, n)

class _Rng:

    def __init__(self, key):
        self._k = key

    def _next(self):
        self._k, sub = jax.random.split(self._k)
        return sub

    def normal(self, shape):
        return jax.random.normal(self._next(), shape, dtype=jnp.bfloat16)

    def randint(self, lo, hi, shape):
        return jax.random.randint(self._next(), shape, lo, hi, dtype=jnp.int32)

    def uniform(self, shape, lo=0.0, hi=1.0):
        return jax.random.uniform(self._next(), shape, jnp.bfloat16, lo, hi)

    def permutation(self, n):
        return jax.random.permutation(self._next(), n)
kernel_name = 'parallel_sum__memory_aug_recurrent_mem_tr__moe_arch_mod__prompt'

def setup_inputs():
    _rng = _Rng(jax.random.key(int.from_bytes(__import__("os").urandom(4), "little")))
    _w = lambda a: (lambda t: t.astype(jnp.bfloat16) if jnp.issubdtype(t.dtype, jnp.floating) else t)(jnp.asarray(a))

    def _A_setup():
        B, S, Dm = (1, 2048, 1024)
        H, Dh = (32, 128)
        M, seg = (8, 32)
        seg = min(seg, S)
        S = S // seg * seg
        return {'x': _w((lambda *s: _rng.normal(s) * 0.05)(B, S, Dm)), 'mem0': _w((lambda *s: _rng.normal(s) * 0.05)(B, M, Dm)), 'Wq': _w((lambda *s: _rng.normal(s) * 0.05)(Dm, H, Dh) * Dm ** (-0.5)), 'Wk': _w((lambda *s: _rng.normal(s) * 0.05)(Dm, H, Dh) * Dm ** (-0.5)), 'Wv': _w((lambda *s: _rng.normal(s) * 0.05)(Dm, H, Dh) * Dm ** (-0.5)), 'Wo': _w((lambda *s: _rng.normal(s) * 0.05)(H, Dh, Dm) * (H * Dh) ** (-0.5)), 'seg_len': seg}
    _A_in = _A_setup()

    def _B_setup():
        B, S, D, F, C = (1, 2048, 1024, 3584, 2)
        return {'x': _w((lambda *s: _rng.normal(s) * 0.05)(B, S, D)), 'w_r': _w((lambda *s: _rng.normal(s) * 0.05)(D)), 'w_gate': _w((lambda *s: _rng.normal(s) * 0.05)(D, F)), 'w_up': _w((lambda *s: _rng.normal(s) * 0.05)(D, F)), 'w_down': _w((lambda *s: _rng.normal(s) * 0.05)(F, D))}
    _B_in = _B_setup()
    return {'A_x': _A_in['x'], 'A_mem0': _A_in['mem0'], 'A_Wq': _A_in['Wq'], 'A_Wk': _A_in['Wk'], 'A_Wv': _A_in['Wv'], 'A_Wo': _A_in['Wo'], 'A_seg_len': _A_in['seg_len'], 'B_x': _B_in['x'], 'B_w_r': _B_in['w_r'], 'B_w_gate': _B_in['w_gate'], 'B_w_up': _B_in['w_up'], 'B_w_down': _B_in['w_down']}

def reference(A_x, A_mem0, A_Wq, A_Wk, A_Wv, A_Wo, A_seg_len, B_x, B_w_r, B_w_gate, B_w_up, B_w_down):

    def _A_ref(x, mem0, Wq, Wk, Wv, Wo, seg_len):
        B, S, Dm = x.shape
        H, Dh = (Wq.shape[1], Wq.shape[2])
        M = mem0.shape[1]
        scale = Dh ** (-0.5)
        n_seg = S // seg_len
        L = M + seg_len
        idx = jnp.arange(L)
        mask = (idx[:, None] < M) | (idx[:, None] >= idx[None, :])
        mem = mem0
        outs = []
        for s in range(n_seg):
            xs = x[:, s * seg_len:(s + 1) * seg_len, :].copy()
            h = jnp.concatenate([mem, xs], axis=1)
            q = jnp.einsum('btd,dhe->bhte', h, Wq)
            k = jnp.einsum('btd,dhe->bhte', h, Wk)
            v = jnp.einsum('btd,dhe->bhte', h, Wv)
            scores = jnp.einsum('bhqe,bhke->bhqk', q, k) * scale
            scores = jnp.where(mask[None, None], scores, -1000000000.0)
            p = _softmax(scores, axis=-1)
            o = jnp.einsum('bhqk,bhke->bhqe', p, v)
            o = jnp.einsum('bhte,hed->btd', o, Wo)
            mem = o[:, :M, :].copy()
            outs.append(o[:, M:, :])
        return jnp.concatenate(outs, axis=1)

    def _B_ref(x, w_r, w_gate, w_up, w_down):
        B, S, D = x.shape
        C = 2
        r = x @ w_r
        idx = jnp.argsort(-r, axis=-1)[:, :C]
        idx_e = jnp.repeat(idx.reshape(B, C, 1), D, axis=2)
        x_sel = jnp.take_along_axis(x, idx_e, axis=1)
        g = _silu(x_sel @ w_gate)
        u = x_sel @ w_up
        y = g * u @ w_down
        r_sel = _sigmoid(jnp.take_along_axis(r, idx, axis=1))
        y = y * r_sel.reshape(B, C, 1)
        b_off = (jnp.arange(B) * S).reshape(B, 1)
        flat_idx = (idx + b_off).reshape(B * C)
        zero = (x * 0.0).reshape(B * S, D)
        upd = _scatter_add(zero, flat_idx, y.reshape(B * C, D), axis=0)
        return x + upd.reshape(B, S, D)
    x = A_x
    xn = _layernorm(x, axis=-1)
    return x + _A_ref(xn, A_mem0, A_Wq, A_Wk, A_Wv, A_Wo, A_seg_len) + _B_ref(xn, B_w_r, B_w_gate, B_w_up, B_w_down)
```

```python
import functools

import jax
import jax.numpy as jnp
import numpy as np
from jax import lax
import jax.experimental.pallas as pl
import jax.experimental.pallas.tpu as pltpu

F32 = jnp.float32
BF16 = jnp.bfloat16
I32 = jnp.int32

_NN = (((1,), (0,)), ((), ()))
_NT = (((1,), (1,)), ((), ()))


def _rb(x):
    return x.astype(BF16).astype(F32)


def _w(ref_words):
    return pltpu.bitcast(ref_words, BF16)


def _dot(a, b, dims=_NN):
    return lax.dot_general(a, b, dims, preferred_element_type=F32)


def _layernorm(x):
    d = x.shape[-1]
    mean = jnp.sum(x, axis=-1, keepdims=True) * (1.0 / d)
    c = x - mean
    var = jnp.sum(c * c, axis=-1, keepdims=True) * (1.0 / d)
    eps = float(np.float32(np.asarray(1e-5, dtype=BF16)))
    den = _rb(jnp.sqrt(_rb(_rb(var) + eps)))
    return _rb(_rb(x - _rb(mean)) / den)


def _kernel(x_hbm, mem0_ref, wq_hbm, wk_hbm, wv_hbm, wo_hbm, wr_ref, wg_hbm, wu_hbm, wd_hbm,
            out_hbm,
            x_v, xn_v, mem_v, o_v, out_v, stage, wq_v, wk_v, wv_v, wo_v, wg_v, wu_v, wd_v,
            top_v,
            sem_x, sem_w, sem_o, sem_f, sem_out, sem_p,
            *, S, D, H, E, M, SEG, F, G):
    n_seg = S // SEG
    L = M + SEG
    HP = H // 2
    scale = float(E) ** -0.5

    cp_x = pltpu.make_async_copy(x_hbm, x_v, sem_x)
    cp_x.start()

    def w_copies(i, w_hbm):
        wi = w_hbm.bitcast(I32)
        return [[pltpu.make_async_copy(wi.at[:, p, j, :], stage.at[i, j, p], sem_w.at[i, 2 * j + p])
                 for p in range(2)] for j in range(HP)]

    w_cps = [w_copies(0, wq_hbm), w_copies(1, wk_hbm), w_copies(2, wv_hbm)]
    for cps in w_cps:
        for pair in cps:
            for c in pair:
                c.start()
    cp_o = pltpu.make_async_copy(wo_hbm.bitcast(I32), wo_v, sem_o)
    cp_o.start()
    cp_f = [pltpu.make_async_copy(wg_hbm.bitcast(I32), wg_v, sem_f.at[0]),
            pltpu.make_async_copy(wu_hbm.bitcast(I32), wu_v, sem_f.at[1]),
            pltpu.make_async_copy(wd_hbm.bitcast(I32), wd_v, sem_f.at[2])]
    for c in cp_f:
        c.start()

    wr = wr_ref[...].astype(F32)

    def ln_segment(s, top):
        row0 = pl.multiple_of(s * SEG, SEG)
        xn = _layernorm(x_v[pl.ds(row0, SEG), :].astype(F32))
        xn_v[pl.ds(row0, SEG), :] = xn
        acc = xn[:, 0:128] * wr[0:1, :]
        for j in range(1, D // 128):
            acc = acc + xn[:, j * 128:(j + 1) * 128] * wr[j:j + 1, :]
        r = _rb(jnp.sum(acc, axis=-1, keepdims=True))
        r = jnp.broadcast_to(r, (SEG, 128))
        v1, i1, v2, i2 = top
        sub = lax.broadcasted_iota(I32, (8, 128), 0)
        for t in range(SEG // 8):
            rv = r[t * 8:(t + 1) * 8]
            ri = sub + (row0 + t * 8)
            gt1 = rv > v1
            gt2 = rv > v2
            v2 = jnp.where(gt1, v1, jnp.where(gt2, rv, v2))
            i2 = jnp.where(gt1, i1, jnp.where(gt2, ri, i2))
            v1 = jnp.where(gt1, rv, v1)
            i1 = jnp.where(gt1, ri, i1)
        return v1, i1, v2, i2

    def load_top():
        return (top_v[0], pltpu.bitcast(top_v[1], I32), top_v[2], pltpu.bitcast(top_v[3], I32))

    def store_top(top):
        v1, i1, v2, i2 = top
        top_v[0] = v1
        top_v[1] = pltpu.bitcast(i1, F32)
        top_v[2] = v2
        top_v[3] = pltpu.bitcast(i2, F32)

    cp_x.wait()
    neg = jnp.full((8, 128), -jnp.inf, F32)
    zero_i = jnp.zeros((8, 128), I32)
    store_top(ln_segment(0, (neg, zero_i, neg, zero_i)))
    mem_v[...] = mem0_ref[...].astype(F32)

    for i, w_v in enumerate((wq_v, wk_v, wv_v)):
        for j in range(HP):
            for c in w_cps[i][j]:
                c.wait()
            a = stage[i, j, 0]
            b = stage[i, j, 1]
            w_v[:, (2 * j) * E:(2 * j + 1) * E] = (a & 0xFFFF) | (b << 16)
            w_v[:, (2 * j + 1) * E:(2 * j + 2) * E] = (
                lax.shift_right_logical(a, 16) | (b & (-65536)))
    cp_o.wait()

    row = lax.broadcasted_iota(I32, (L, L), 0)
    col = lax.broadcasted_iota(I32, (L, L), 1)
    mask = (row < M) | (row >= col)

    def step(s, carry):
        row0 = pl.multiple_of(s * SEG, SEG)

        def h():
            return jnp.concatenate([mem_v[...], xn_v[pl.ds(row0, SEG), :]], axis=0)

        for g in range(H // G):
            cols = slice(g * G * E, (g + 1) * G * E)
            q = _dot(h(), _w(wq_v[:, cols]))
            k = _dot(h(), _w(wk_v[:, cols]))
            v = _dot(h(), _w(wv_v[:, cols]))
            for u in range(G):
                hs = slice(u * E, (u + 1) * E)
                sc = _dot(q[:, hs], k[:, hs], _NT) * scale
                sc = jnp.where(mask, sc, -1e9)
                e = jnp.exp(sc - jnp.max(sc, axis=-1, keepdims=True))
                p = e / jnp.sum(e, axis=-1, keepdims=True)
                o_v[:, (g * G + u) * E:(g * G + u + 1) * E] = _dot(p, v[:, hs])
        y = _dot(o_v[...], _w(wo_v[...]))
        mem_v[...] = y[0:M]
        res = x_v[pl.ds(row0, SEG), :].astype(F32) + xn_v[pl.ds(row0, SEG), :] + y[M:]
        out_v[pl.ds(row0, SEG), :] = res.astype(BF16)
        pltpu.make_async_copy(out_v.at[pl.ds(row0, SEG), :], out_hbm.at[pl.ds(row0, SEG), :],
                              sem_out).start()
        store_top(ln_segment(jnp.minimum(s + 1, n_seg - 1), load_top()))
        return carry

    lax.fori_loop(0, n_seg, step, 0)

    v1, i1, v2, i2 = load_top()
    big = jnp.int32(2 ** 30)
    m1 = jnp.max(v1, axis=0, keepdims=True)
    j1 = jnp.min(jnp.where(v1 == m1, i1, big), axis=0, keepdims=True)
    hit = i1 == j1
    c_v = jnp.where(hit, v2, v1)
    c_i = jnp.where(hit, i2, i1)
    m2 = jnp.max(c_v, axis=0, keepdims=True)
    j2 = jnp.min(jnp.where(c_v == m2, c_i, big), axis=0, keepdims=True)
    t1 = jnp.clip(j1[0, 0], 0, S - 1)
    t2 = jnp.clip(j2[0, 0], 0, S - 1)

    sub = lax.broadcasted_iota(I32, (8, D), 0)
    xs = jnp.where(sub == 0, xn_v[pl.ds(t1, 1), :], xn_v[pl.ds(t2, 1), :])
    for c in cp_f:
        c.wait()
    gate = _dot(xs, _w(wg_v[...]))
    up = _dot(xs, _w(wu_v[...]))
    act = gate * jax.nn.sigmoid(gate) * up
    yf = _dot(act, _w(wd_v[...]))
    sub1 = lax.broadcasted_iota(I32, (8, 128), 0)
    rs = jax.nn.sigmoid(jnp.where(sub1 == 0, m1, m2))
    yf = yf * rs[:, 0:1]

    pltpu.make_async_copy(out_v, out_v, sem_out).wait()

    rows16 = lax.broadcasted_iota(I32, (16, D), 0)
    b1 = pl.multiple_of((t1 // 16) * 16, 16)
    b2 = pl.multiple_of((t2 // 16) * 16, 16)
    blk = out_v[pl.ds(b1, 16), :].astype(F32)
    out_v[pl.ds(b1, 16), :] = jnp.where(rows16 == t1 - b1, blk + yf[0:1], blk).astype(BF16)
    blk = out_v[pl.ds(b2, 16), :].astype(F32)
    out_v[pl.ds(b2, 16), :] = jnp.where(rows16 == t2 - b2, blk + yf[1:2], blk).astype(BF16)

    cp1 = pltpu.make_async_copy(out_v.at[pl.ds(b1, 16), :], out_hbm.at[pl.ds(b1, 16), :], sem_p.at[0])
    cp1.start()

    @pl.when(b1 != b2)
    def _():
        cp2 = pltpu.make_async_copy(out_v.at[pl.ds(b2, 16), :], out_hbm.at[pl.ds(b2, 16), :],
                                    sem_p.at[1])
        cp2.start()
        cp2.wait()

    cp1.wait()


@functools.partial(jax.jit, static_argnames=("A_seg_len",))
def pallas_parallel_sum__memory_aug_recurrent_mem_tr__moe_arch_mod__prompt_kernel(
    A_x, A_mem0, A_Wq, A_Wk, A_Wv, A_Wo, A_seg_len, B_x, B_w_r, B_w_gate, B_w_up, B_w_down,
):
    del B_x
    B, S, D = A_x.shape
    _, H, E = A_Wq.shape
    M = A_mem0.shape[1]
    F = B_w_gate.shape[1]
    SEG = int(A_seg_len)
    assert B == 1
    L = M + SEG
    any_spec = pl.BlockSpec(memory_space=pl.ANY)
    vmem_spec = pl.BlockSpec(memory_space=pltpu.VMEM)
    kern = functools.partial(_kernel, S=S, D=D, H=H, E=E, M=M, SEG=SEG, F=F, G=4)
    out = pl.pallas_call(
        kern,
        out_shape=jax.ShapeDtypeStruct((S, D), A_x.dtype),
        in_specs=[any_spec, vmem_spec, any_spec, any_spec, any_spec, any_spec, vmem_spec,
                  any_spec, any_spec, any_spec],
        out_specs=any_spec,
        scratch_shapes=[
            pltpu.VMEM((S, D), BF16),
            pltpu.VMEM((S, D), F32),
            pltpu.VMEM((M, D), F32),
            pltpu.VMEM((L, H * E), F32),
            pltpu.VMEM((S, D), BF16),
            pltpu.VMEM((3, H // 2, 2, D // 2, E), I32),
            pltpu.VMEM((D // 2, H * E), I32),
            pltpu.VMEM((D // 2, H * E), I32),
            pltpu.VMEM((D // 2, H * E), I32),
            pltpu.VMEM((H * E // 2, D), I32),
            pltpu.VMEM((D // 2, F), I32),
            pltpu.VMEM((D // 2, F), I32),
            pltpu.VMEM((F // 2, D), I32),
            pltpu.VMEM((4, 8, 128), F32),
            pltpu.SemaphoreType.DMA(()),
            pltpu.SemaphoreType.DMA((3, H)),
            pltpu.SemaphoreType.DMA(()),
            pltpu.SemaphoreType.DMA((3,)),
            pltpu.SemaphoreType.DMA(()),
            pltpu.SemaphoreType.DMA((2,)),
        ],
        compiler_params=pltpu.CompilerParams(vmem_limit_bytes=120 * 1024 * 1024),
    )(
        A_x.reshape(S, D), A_mem0.reshape(M, D),
        A_Wq.reshape(D // 2, 2, H, E), A_Wk.reshape(D // 2, 2, H, E), A_Wv.reshape(D // 2, 2, H, E),
        A_Wo.reshape(H * E, D), B_w_r.reshape(D // 128, 128), B_w_gate, B_w_up, B_w_down,
    )
    return out.reshape(B, S, D)
```

```python
import functools

import jax
import jax.numpy as jnp
import numpy as np
from jax import lax
import jax.experimental.pallas as pl
import jax.experimental.pallas.tpu as pltpu

F32 = jnp.float32
BF16 = jnp.bfloat16
I32 = jnp.int32

_NN = (((1,), (0,)), ((), ()))
_NT = (((1,), (1,)), ((), ()))


def _rb(x):
    return x.astype(BF16).astype(F32)


def _w(words):
    return pltpu.bitcast(words, BF16)


def _dot(a, b, dims=_NN):
    return lax.dot_general(a, b, dims, preferred_element_type=F32)


def _layernorm(x):
    d = x.shape[-1]
    mean = jnp.sum(x, axis=-1, keepdims=True) * (1.0 / d)
    c = x - mean
    var = jnp.sum(c * c, axis=-1, keepdims=True) * (1.0 / d)
    eps = float(np.float32(np.asarray(1e-5, dtype=BF16)))
    den = _rb(jnp.sqrt(_rb(_rb(var) + eps)))
    return _rb(_rb(x - _rb(mean)) / den)


def _kernel(x_hbm, mem0_ref, wq_hbm, wk_hbm, wv_hbm, wo_hbm, wr_ref, wg_hbm, wu_hbm, wd_hbm,
            out_hbm,
            x_v, xn_v, mem_v, o_v, out_v, wq_v, wk_v, wv_v, wo_v, wg_v, wu_v, wd_v,
            rq_v, rk_v, rv_v, top_v, yf_v,
            sem_x, sem_w, sem_o, sem_f, sem_out,
            *, S, D, H, E, M, SEG, F, G, T, R0, RING, OFF):
    n_seg = S // SEG
    L = M + SEG
    NG = H // G
    XC = (S - R0) // NG
    scale = float(E) ** -0.5
    w_hbm = (wq_hbm, wk_hbm, wv_hbm)
    w_vm = (wq_v, wk_v, wv_v)
    ring = (rq_v, rk_v, rv_v)

    FC = F // (NG - 1)

    def x_copy(c):
        if isinstance(c, int) and c == 0:
            rows = pl.ds(0, R0)
        else:
            rows = pl.ds(pl.multiple_of(R0 + (c - 1) * XC, 16), XC)
        return pltpu.make_async_copy(x_hbm.at[rows], x_v.at[rows], sem_x.at[c])

    def start_group(g):
        for m in range(3):
            for u in range(G):
                pltpu.make_async_copy(
                    w_hbm[m].bitcast(I32).at[:, u % 2, g * (G // 2) + u // 2, :],
                    w_vm[m].at[g * G + u], sem_w.at[m, g]).start()

    def start_ffn(c):
        cols = pl.ds(pl.multiple_of(c * FC, 128), FC)
        rows = pl.ds(pl.multiple_of(c * (FC // 2), 8), FC // 2)
        pltpu.make_async_copy(wg_hbm.bitcast(I32).at[:, cols], wg_v.at[:, cols], sem_f.at[0]).start()
        pltpu.make_async_copy(wu_hbm.bitcast(I32).at[:, cols], wu_v.at[:, cols], sem_f.at[1]).start()
        pltpu.make_async_copy(wd_hbm.bitcast(I32).at[rows, :], wd_v.at[rows, :], sem_f.at[2]).start()

    cp_o = pltpu.make_async_copy(wo_hbm.bitcast(I32), wo_v, sem_o)
    x_copy(0).start()

    def ln_rows(row0, n):
        wr = wr_ref[...].astype(F32)
        xn = _layernorm(x_v[pl.ds(row0, n), :].astype(F32))
        xn_v[pl.ds(row0, n), :] = xn
        acc = xn[:, 0:128] * wr[0:1, :]
        for j in range(1, D // 128):
            acc = acc + xn[:, j * 128:(j + 1) * 128] * wr[j:j + 1, :]
        r = jnp.broadcast_to(_rb(jnp.sum(acc, axis=-1, keepdims=True)), (n, 128))
        v1, v2 = top_v[0], top_v[2]
        i1, i2 = pltpu.bitcast(top_v[1], I32), pltpu.bitcast(top_v[3], I32)
        sub = lax.broadcasted_iota(I32, (8, 128), 0)
        for t in range(n // 8):
            rv = r[t * 8:(t + 1) * 8]
            ri = sub + (row0 + t * 8)
            gt1 = rv > v1
            gt2 = rv > v2
            v2 = jnp.where(gt1, v1, jnp.where(gt2, rv, v2))
            i2 = jnp.where(gt1, i1, jnp.where(gt2, ri, i2))
            v1 = jnp.where(gt1, rv, v1)
            i1 = jnp.where(gt1, ri, i1)
        top_v[0] = v1
        top_v[1] = pltpu.bitcast(i1, F32)
        top_v[2] = v2
        top_v[3] = pltpu.bitcast(i2, F32)

    neg = jnp.full((8, 128), -jnp.inf, F32)
    top_v[0] = neg
    top_v[2] = neg
    top_v[1] = jnp.zeros((8, 128), F32)
    top_v[3] = jnp.zeros((8, 128), F32)
    mem_v[...] = mem0_ref[...].astype(F32)

    x_copy(0).wait()
    start_group(0)
    x_copy(1).start()
    LNB = 64

    def ln_body(i, c):
        ln_rows(pl.multiple_of(i * LNB, LNB), LNB)
        return c

    lax.fori_loop(0, R0 // LNB, ln_body, 0)

    def pro_body(g, c):
        @pl.when(g < NG - 1)
        def _():
            start_group(g + 1)
            x_copy(g + 2).start()
            start_ffn(g)

        @pl.when(g == NG - 1)
        def _():
            cp_o.start()

        grp = pl.ds(pl.multiple_of(g * G, G), G)
        for m in range(3):
            pltpu.make_async_copy(w_vm[m].at[grp], w_vm[m].at[grp], sem_w.at[m, g]).wait()
        x_copy(g + 1).wait()
        for m in range(3):
            ws = []
            for u in range(0, G, 2):
                a = w_vm[m][g * G + u]
                b = w_vm[m][g * G + u + 1]
                lo = (a & 0xFFFF) | (b << 16)
                hi = lax.shift_right_logical(a, 16) | (b & (-65536))
                w_vm[m][g * G + u] = lo
                w_vm[m][g * G + u + 1] = hi
                ws += [lo, hi]
            ring[m][g, pl.ds(OFF, R0), :] = _dot(xn_v[0:R0, :], _w(jnp.concatenate(ws, axis=1)))
        ln_rows(pl.multiple_of(R0 + g * XC, 16), XC)
        return c

    lax.fori_loop(0, NG, pro_body, 0)

    v1, v2 = top_v[0], top_v[2]
    i1, i2 = pltpu.bitcast(top_v[1], I32), pltpu.bitcast(top_v[3], I32)
    big = 2 ** 30
    m1 = jnp.max(v1, axis=0, keepdims=True)
    j1 = jnp.min(jnp.where(v1 == m1, i1, big), axis=0, keepdims=True)
    hit = i1 == j1
    c_v = jnp.where(hit, v2, v1)
    c_i = jnp.where(hit, i2, i1)
    m2 = jnp.max(c_v, axis=0, keepdims=True)
    j2 = jnp.min(jnp.where(c_v == m2, c_i, big), axis=0, keepdims=True)
    t1 = jnp.clip(j1[0, 0], 0, S - 1)
    t2 = jnp.clip(j2[0, 0], 0, S - 1)

    sub = lax.broadcasted_iota(I32, (8, D), 0)
    xs = jnp.where(sub == 0, xn_v[pl.ds(t1, 1), :], xn_v[pl.ds(t2, 1), :])
    for i, w in enumerate((wg_v, wu_v, wd_v)):
        pltpu.make_async_copy(w, w, sem_f.at[i]).wait()
    gate = _dot(xs, _w(wg_v[...]))
    up = _dot(xs, _w(wu_v[...]))
    act = gate * jax.nn.sigmoid(gate) * up
    yf = _dot(act, _w(wd_v[...]))
    sub1 = lax.broadcasted_iota(I32, (8, 128), 0)
    rs = jax.nn.sigmoid(jnp.where(sub1 == 0, m1, m2))
    yf_v[...] = yf * rs[:, 0:1]
    cp_o.wait()

    row = lax.broadcasted_iota(I32, (L, L), 0)
    col = lax.broadcasted_iota(I32, (L, L), 1)
    mask = (row < M) | (row >= col)
    hs = lambda u: slice(u * E, (u + 1) * E)

    def step(s, carry):
        row0 = pl.multiple_of(s * SEG, SEG)
        new0 = pl.multiple_of(R0 + s * T, 8)
        wr0 = pl.multiple_of(lax.rem(R0 + OFF + s * T, RING), 8)
        rd0 = pl.multiple_of(lax.rem(OFF + s * SEG, RING), SEG)

        def proj(m, g):
            h = jnp.concatenate([mem_v[...], xn_v[pl.ds(new0, T), :]], axis=0)
            w = jnp.concatenate([w_vm[m][g * G + u] for u in range(G)], axis=1)
            y = _dot(h, _w(w))
            ring[m][g, pl.ds(wr0, T), :] = y[M:]
            return y[0:M]

        def seg_rows(m, g, mem_rows):
            return jnp.concatenate([mem_rows, ring[m][g, pl.ds(rd0, SEG), :]], axis=0)

        def scores(g, qm, km):
            q = seg_rows(0, g, qm)
            k = seg_rows(1, g, km)
            ps = []
            for u in range(G):
                sc = _dot(q[:, hs(u)], k[:, hs(u)], _NT) * scale
                sc = jnp.where(mask, sc, -1e9)
                e = jnp.exp(sc - jnp.max(sc, axis=-1, keepdims=True))
                ps.append(e / jnp.sum(e, axis=-1, keepdims=True))
            return ps

        def attend(g, ps, vm):
            v = seg_rows(2, g, vm)
            for u in range(G):
                o_v[:, (g * G + u) * E:(g * G + u + 1) * E] = _dot(ps[u], v[:, hs(u)])

        def outproj(g0, g1):
            return _dot(o_v[:, g0 * G * E:g1 * G * E],
                        _w(wo_v[g0 * G * E // 2:g1 * G * E // 2, :]))

        prev = None
        for g in range(NG):
            qm = proj(0, g)
            km = proj(1, g)
            if prev is not None:
                attend(g - 1, *prev)
            vm = proj(2, g)
            prev = (scores(g, qm, km), vm)
        y = outproj(0, NG - 2)
        attend(NG - 1, *prev)
        y = outproj(NG - 2, NG - 1) + y
        y = outproj(NG - 1, NG) + y
        mem_v[...] = y[0:M]
        tok = lax.broadcasted_iota(I32, (SEG, D), 0) + row0
        upd = (jnp.where(tok == t1, yf_v[0:1, :], 0.0) + jnp.where(tok == t2, yf_v[1:2, :], 0.0))
        res = (x_v[pl.ds(row0, SEG), :].astype(F32) + y[M:]) + (xn_v[pl.ds(row0, SEG), :] + upd)
        out_v[pl.ds(row0, SEG), :] = res.astype(BF16)
        pltpu.make_async_copy(out_v.at[pl.ds(row0, SEG), :], out_hbm.at[pl.ds(row0, SEG), :],
                              sem_out).start()
        return carry

    lax.fori_loop(0, n_seg, step, 0)
    pltpu.make_async_copy(out_v, out_v, sem_out).wait()


@functools.partial(jax.jit, static_argnames=("A_seg_len",))
def pallas_parallel_sum__memory_aug_recurrent_mem_tr__moe_arch_mod__prompt_kernel(
    A_x, A_mem0, A_Wq, A_Wk, A_Wv, A_Wo, A_seg_len, B_x, B_w_r, B_w_gate, B_w_up, B_w_down,
):
    del B_x
    B, S, D = A_x.shape
    _, H, E = A_Wq.shape
    M = A_mem0.shape[1]
    F = B_w_gate.shape[1]
    SEG = int(A_seg_len)
    assert B == 1
    L = M + SEG
    G = 4
    NG = H // G
    T = 24
    R0 = S - (S // SEG) * T
    RING, OFF = 576, 64
    assert (R0 + OFF) % T == 0 and OFF % SEG == 0 and RING % T == 0 and RING % SEG == 0
    assert R0 + OFF <= RING and R0 + T <= RING
    any_spec = pl.BlockSpec(memory_space=pl.ANY)
    vmem_spec = pl.BlockSpec(memory_space=pltpu.VMEM)
    kern = functools.partial(_kernel, S=S, D=D, H=H, E=E, M=M, SEG=SEG, F=F, G=G, T=T, R0=R0,
                             RING=RING, OFF=OFF)
    out = pl.pallas_call(
        kern,
        out_shape=jax.ShapeDtypeStruct((S, D), A_x.dtype),
        in_specs=[any_spec, vmem_spec, any_spec, any_spec, any_spec, any_spec, vmem_spec,
                  any_spec, any_spec, any_spec],
        out_specs=any_spec,
        scratch_shapes=[
            pltpu.VMEM((S, D), BF16),
            pltpu.VMEM((S, D), F32),
            pltpu.VMEM((M, D), F32),
            pltpu.VMEM((L, H * E), F32),
            pltpu.VMEM((S, D), BF16),
            pltpu.VMEM((H, D // 2, E), I32),
            pltpu.VMEM((H, D // 2, E), I32),
            pltpu.VMEM((H, D // 2, E), I32),
            pltpu.VMEM((H * E // 2, D), I32),
            pltpu.VMEM((D // 2, F), I32),
            pltpu.VMEM((D // 2, F), I32),
            pltpu.VMEM((F // 2, D), I32),
            pltpu.VMEM((NG, RING, G * E), F32),
            pltpu.VMEM((NG, RING, G * E), F32),
            pltpu.VMEM((NG, RING, G * E), F32),
            pltpu.VMEM((4, 8, 128), F32),
            pltpu.VMEM((8, D), F32),
            pltpu.SemaphoreType.DMA((NG + 1,)),
            pltpu.SemaphoreType.DMA((3, NG)),
            pltpu.SemaphoreType.DMA(()),
            pltpu.SemaphoreType.DMA((3,)),
            pltpu.SemaphoreType.DMA(()),
        ],
        compiler_params=pltpu.CompilerParams(vmem_limit_bytes=120 * 1024 * 1024),
    )(
        A_x.reshape(S, D), A_mem0.reshape(M, D),
        A_Wq.reshape(D // 2, 2, H, E), A_Wk.reshape(D // 2, 2, H, E), A_Wv.reshape(D // 2, 2, H, E),
        A_Wo.reshape(H * E, D), B_w_r.reshape(D // 128, 128), B_w_gate, B_w_up, B_w_down,
    )
    return out.reshape(B, S, D)
```

```python
import functools

import jax
import jax.numpy as jnp
import numpy as np
from jax import lax
import jax.experimental.pallas as pl
import jax.experimental.pallas.tpu as pltpu

F32 = jnp.float32
BF16 = jnp.bfloat16
I32 = jnp.int32

_NN = (((1,), (0,)), ((), ()))
_NT = (((1,), (1,)), ((), ()))


def _rb(x):
    return x.astype(BF16).astype(F32)


def _w(words):
    return pltpu.bitcast(words, BF16)


def _dot(a, b, dims=_NN):
    return lax.dot_general(a, b, dims, preferred_element_type=F32)


def _layernorm(x):
    d = x.shape[-1]
    mean = jnp.sum(x, axis=-1, keepdims=True) * (1.0 / d)
    c = x - mean
    var = jnp.sum(c * c, axis=-1, keepdims=True) * (1.0 / d)
    eps = float(np.float32(np.asarray(1e-5, dtype=BF16)))
    den = _rb(jnp.sqrt(_rb(_rb(var) + eps)))
    return _rb(_rb(x - _rb(mean)) / den)


def _kernel(x_hbm, mem0_ref, wq_hbm, wk_hbm, wv_hbm, wo_hbm, wr_ref, wg_hbm, wu_hbm, wd_hbm,
            out_hbm,
            x_v, xn_v, mem_v, o_v, out_v, wq_v, wk_v, wv_v, wo_v, wg_v, wu_v, wd_v,
            rq_v, rk_v, rv_v, r_v, yf_v, p_v, mq_v, mk_v, mv_v, h_v, xh_v,
            sem_x, sem_w, sem_o, sem_f, sem_out,
            *, S, D, H, E, M, SEG, F, G, T, R0, RING, OFF):
    n_seg = S // SEG
    L = M + SEG
    NG = H // G
    XC = (S - R0) // NG
    scale = float(E) ** -0.5
    w_hbm = (wq_hbm, wk_hbm, wv_hbm)
    w_vm = (wq_v, wk_v, wv_v)
    ring = (rq_v, rk_v, rv_v)

    FC = F // (NG - 1)

    def x_copy(c):
        if isinstance(c, int) and c == 0:
            rows = pl.ds(0, R0)
        else:
            rows = pl.ds(pl.multiple_of(R0 + (c - 1) * XC, 16), XC)
        return pltpu.make_async_copy(x_hbm.at[rows], x_v.at[rows], sem_x.at[c])

    def start_group(g):
        for m in range(3):
            for u in range(G):
                pltpu.make_async_copy(
                    w_hbm[m].bitcast(I32).at[:, u % 2, g * (G // 2) + u // 2, :],
                    w_vm[m].at[g * G + u], sem_w.at[m, g]).start()

    def start_ffn(c):
        cols = pl.ds(pl.multiple_of(c * FC, 128), FC)
        rows = pl.ds(pl.multiple_of(c * (FC // 2), 8), FC // 2)
        pltpu.make_async_copy(wg_hbm.bitcast(I32).at[:, cols], wg_v.at[:, cols], sem_f.at[0]).start()
        pltpu.make_async_copy(wu_hbm.bitcast(I32).at[:, cols], wu_v.at[:, cols], sem_f.at[1]).start()
        pltpu.make_async_copy(wd_hbm.bitcast(I32).at[rows, :], wd_v.at[rows, :], sem_f.at[2]).start()

    cp_o = pltpu.make_async_copy(wo_hbm.bitcast(I32), wo_v, sem_o)
    x_copy(0).start()

    def ln_rows(row0, n, slab, packed=False):
        wr = wr_ref[...].astype(F32)
        xn = _layernorm(x_v[pl.ds(row0, n), :].astype(F32))
        xn_v[pl.ds(row0, n), :] = xn
        if packed:
            xh_v[pl.ds(pl.multiple_of(row0 // 2, n // 2), n // 2), :] = pltpu.bitcast(xn.astype(BF16), I32)
        acc = xn[:, 0:128] * wr[0:1, :]
        for j in range(1, D // 128):
            acc = acc + xn[:, j * 128:(j + 1) * 128] * wr[j:j + 1, :]
        r = jnp.broadcast_to(_rb(jnp.sum(acc, axis=-1, keepdims=True)), (n, 128))
        lane = lax.broadcasted_iota(I32, (8, 128), 1)
        slab_r = jnp.full((8, 128), -jnp.inf, F32)
        for t in range(n // 8):
            slab_r = jnp.where(lane == t, r[t * 8:(t + 1) * 8], slab_r)
        r_v[slab] = slab_r

    mem_v[...] = mem0_ref[...].astype(F32)

    x_copy(0).wait()
    start_group(0)
    x_copy(1).start()
    LNB = 64

    def ln_body(i, c):
        ln_rows(pl.multiple_of(i * LNB, LNB), LNB, NG + i, packed=True)
        return c

    lax.fori_loop(0, R0 // LNB, ln_body, 0)

    def pro_body(g, c):
        @pl.when(g < NG - 1)
        def _():
            start_group(g + 1)
            x_copy(g + 2).start()
            start_ffn(g)

        @pl.when(g == NG - 1)
        def _():
            cp_o.start()

        grp = pl.ds(pl.multiple_of(g * G, G), G)
        for m in range(3):
            pltpu.make_async_copy(w_vm[m].at[grp], w_vm[m].at[grp], sem_w.at[m, g]).wait()
        x_copy(g + 1).wait()
        ln_rows(pl.multiple_of(R0 + g * XC, 16), XC, g)
        for m in range(3):
            ws = []
            for u in range(0, G, 2):
                a = w_vm[m][g * G + u]
                b = w_vm[m][g * G + u + 1]
                lo = (a & 0xFFFF) | (b << 16)
                hi = lax.shift_right_logical(a, 16) | (b & (-65536))
                w_vm[m][g * G + u] = lo
                w_vm[m][g * G + u + 1] = hi
                ws += [lo, hi]
            ring[m][g, pl.ds(OFF, R0), :] = _dot(_w(xh_v[...]), _w(jnp.concatenate(ws, axis=1)))
        return c

    lax.fori_loop(0, NG, pro_body, 0)

    pos = (lax.broadcasted_iota(I32, (8, 128), 1) * 8 + lax.broadcasted_iota(I32, (8, 128), 0))
    bases = [R0 + g * XC for g in range(NG)] + [i * LNB for i in range(R0 // LNB)]
    vals = [r_v[i] for i in range(len(bases))]
    toks = [(pos + b).astype(F32) for b in bases]

    def all_max(vs):
        m = functools.reduce(jnp.maximum, vs)
        return jnp.max(jnp.max(m, axis=0, keepdims=True), axis=1, keepdims=True)

    def first_with(vs, m):
        c = functools.reduce(jnp.minimum, [jnp.where(v == m, t, float(S)) for v, t in zip(vs, toks)])
        return jnp.min(jnp.min(c, axis=0, keepdims=True), axis=1, keepdims=True)

    m1 = all_max(vals)
    j1 = first_with(vals, m1)
    vals = [jnp.where(t == j1, -jnp.inf, v) for v, t in zip(vals, toks)]
    m2 = all_max(vals)
    j2 = first_with(vals, m2)
    j1 = j1.astype(I32)
    j2 = j2.astype(I32)
    t1 = jnp.clip(j1[0, 0], 0, S - 1)
    t2 = jnp.clip(j2[0, 0], 0, S - 1)

    sub = lax.broadcasted_iota(I32, (8, D), 0)
    xs = jnp.where(sub == 0, xn_v[pl.ds(t1, 1), :], xn_v[pl.ds(t2, 1), :])
    for i, w in enumerate((wg_v, wu_v, wd_v)):
        pltpu.make_async_copy(w, w, sem_f.at[i]).wait()
    gate = _dot(xs, _w(wg_v[...]))
    up = _dot(xs, _w(wu_v[...]))
    act = gate * jax.nn.sigmoid(gate) * up
    yf = _dot(act, _w(wd_v[...]))
    sub1 = lax.broadcasted_iota(I32, (8, 128), 0)
    rs = jax.nn.sigmoid(jnp.where(sub1 == 0, m1, m2))
    yf_v[...] = yf * rs[:, 0:1]
    cp_o.wait()

    row = lax.broadcasted_iota(I32, (L, L), 0)
    col = lax.broadcasted_iota(I32, (L, L), 1)
    mask = (row < M) | (row >= col)
    hs = lambda u: slice(u * E, (u + 1) * E)

    def step(s, carry):
        row0 = pl.multiple_of(s * SEG, SEG)
        new0 = pl.multiple_of(R0 + s * T, 8)
        wr0 = pl.multiple_of(lax.rem(R0 + OFF + s * T, RING), 8)
        rd0 = pl.multiple_of(lax.rem(OFF + s * SEG, RING), SEG)

        mrow = (mq_v, mk_v, mv_v)
        h_v[...] = pltpu.bitcast(
            jnp.concatenate([mem_v[...], xn_v[pl.ds(new0, T), :]], axis=0).astype(BF16), I32)

        def proj(m, g):
            h = _w(h_v[...])
            w = jnp.concatenate([w_vm[m][g * G + u] for u in range(G)], axis=1)
            y = _dot(h, _w(w))
            ring[m][g, pl.ds(wr0, T), :] = y[M:]
            mrow[m][g % 2] = y[0:M]

        def seg_rows(m, g):
            return jnp.concatenate([mrow[m][g % 2], ring[m][g, pl.ds(rd0, SEG), :]], axis=0)

        def scores(g):
            q = seg_rows(0, g)
            k = seg_rows(1, g)
            for u in range(G):
                sc = _dot(q[:, hs(u)], k[:, hs(u)], _NT) * scale
                sc = jnp.where(mask, sc, -1e9)
                e = jnp.exp(sc - jnp.max(sc, axis=-1, keepdims=True))
                p_v[g % 2, u] = e / jnp.sum(e, axis=-1, keepdims=True)

        def attend(g):
            v = seg_rows(2, g)
            for u in range(G):
                o_v[:, (g * G + u) * E:(g * G + u + 1) * E] = _dot(p_v[g % 2, u], v[:, hs(u)])

        def outproj(g0, g1):
            return _dot(o_v[:, g0 * G * E:g1 * G * E],
                        _w(wo_v[g0 * G * E // 2:g1 * G * E // 2, :]))

        for g in range(NG):
            proj(0, g)
            proj(1, g)
            if g > 0:
                attend(g - 1)
            proj(2, g)
            scores(g)
        y = outproj(0, NG - 2)
        attend(NG - 1)
        y = outproj(NG - 2, NG - 1) + y
        y = outproj(NG - 1, NG) + y
        mem_v[...] = y[0:M]
        tok = lax.broadcasted_iota(I32, (SEG, D), 0) + row0
        upd = (jnp.where(tok == t1, yf_v[0:1, :], 0.0) + jnp.where(tok == t2, yf_v[1:2, :], 0.0))
        res = (x_v[pl.ds(row0, SEG), :].astype(F32) + y[M:]) + (xn_v[pl.ds(row0, SEG), :] + upd)
        out_v[pl.ds(row0, SEG), :] = res.astype(BF16)
        pltpu.make_async_copy(out_v.at[pl.ds(row0, SEG), :], out_hbm.at[pl.ds(row0, SEG), :],
                              sem_out).start()
        return carry

    lax.fori_loop(0, n_seg, step, 0)
    pltpu.make_async_copy(out_v, out_v, sem_out).wait()


@functools.partial(jax.jit, static_argnames=("A_seg_len",))
def pallas_parallel_sum__memory_aug_recurrent_mem_tr__moe_arch_mod__prompt_kernel(
    A_x, A_mem0, A_Wq, A_Wk, A_Wv, A_Wo, A_seg_len, B_x, B_w_r, B_w_gate, B_w_up, B_w_down,
):
    del B_x
    B, S, D = A_x.shape
    _, H, E = A_Wq.shape
    M = A_mem0.shape[1]
    F = B_w_gate.shape[1]
    SEG = int(A_seg_len)
    assert B == 1
    L = M + SEG
    G = 4
    NG = H // G
    T = 24
    R0 = S - (S // SEG) * T
    RING, OFF = 576, 64
    assert (R0 + OFF) % T == 0 and OFF % SEG == 0 and RING % T == 0 and RING % SEG == 0
    assert R0 + OFF <= RING and R0 + T <= RING
    any_spec = pl.BlockSpec(memory_space=pl.ANY)
    vmem_spec = pl.BlockSpec(memory_space=pltpu.VMEM)
    kern = functools.partial(_kernel, S=S, D=D, H=H, E=E, M=M, SEG=SEG, F=F, G=G, T=T, R0=R0,
                             RING=RING, OFF=OFF)
    out = pl.pallas_call(
        kern,
        out_shape=jax.ShapeDtypeStruct((S, D), A_x.dtype),
        in_specs=[any_spec, vmem_spec, any_spec, any_spec, any_spec, any_spec, vmem_spec,
                  any_spec, any_spec, any_spec],
        out_specs=any_spec,
        scratch_shapes=[
            pltpu.VMEM((S, D), BF16),
            pltpu.VMEM((S, D), F32),
            pltpu.VMEM((M, D), F32),
            pltpu.VMEM((L, H * E), F32),
            pltpu.VMEM((S, D), BF16),
            pltpu.VMEM((H, D // 2, E), I32),
            pltpu.VMEM((H, D // 2, E), I32),
            pltpu.VMEM((H, D // 2, E), I32),
            pltpu.VMEM((H * E // 2, D), I32),
            pltpu.VMEM((D // 2, F), I32),
            pltpu.VMEM((D // 2, F), I32),
            pltpu.VMEM((F // 2, D), I32),
            pltpu.VMEM((NG, RING, G * E), F32),
            pltpu.VMEM((NG, RING, G * E), F32),
            pltpu.VMEM((NG, RING, G * E), F32),
            pltpu.VMEM((NG + R0 // 64, 8, 128), F32),
            pltpu.VMEM((8, D), F32),
            pltpu.VMEM((2, G, L, L), F32),
            pltpu.VMEM((2, M, G * E), F32),
            pltpu.VMEM((2, M, G * E), F32),
            pltpu.VMEM((2, M, G * E), F32),
            pltpu.VMEM(((M + T) // 2, D), I32),
            pltpu.VMEM((R0 // 2, D), I32),
            pltpu.SemaphoreType.DMA((NG + 1,)),
            pltpu.SemaphoreType.DMA((3, NG)),
            pltpu.SemaphoreType.DMA(()),
            pltpu.SemaphoreType.DMA((3,)),
            pltpu.SemaphoreType.DMA(()),
        ],
        compiler_params=pltpu.CompilerParams(vmem_limit_bytes=120 * 1024 * 1024),
    )(
        A_x.reshape(S, D), A_mem0.reshape(M, D),
        A_Wq.reshape(D // 2, 2, H, E), A_Wk.reshape(D // 2, 2, H, E), A_Wv.reshape(D // 2, 2, H, E),
        A_Wo.reshape(H * E, D), B_w_r.reshape(D // 128, 128), B_w_gate, B_w_up, B_w_down,
    )
    return out.reshape(B, S, D)
```

```python
import functools

import jax
import jax.numpy as jnp
import numpy as np
from jax import lax
import jax.experimental.pallas as pl
import jax.experimental.pallas.tpu as pltpu

F32 = jnp.float32
BF16 = jnp.bfloat16
I32 = jnp.int32

_LOG2E = float(np.log2(np.e))
_NN = (((1,), (0,)), ((), ()))
_NT = (((1,), (1,)), ((), ()))


def _rb(x):
    return x.astype(BF16).astype(F32)


def _w(words):
    return pltpu.bitcast(words, BF16)


def _dot(a, b, dims=_NN):
    return lax.dot_general(a, b, dims, preferred_element_type=F32)


def _recip(x):
    r = pl.reciprocal(x, approx=True)
    return r * (2.0 - x * r)


def _layernorm(x):
    d = x.shape[-1]
    mean = jnp.sum(x, axis=-1, keepdims=True) * (1.0 / d)
    c = x - mean
    var = jnp.sum(c * c, axis=-1, keepdims=True) * (1.0 / d)
    eps = float(np.float32(np.asarray(1e-5, dtype=BF16)))
    den = _rb(jnp.sqrt(_rb(_rb(var) + eps)))
    return _rb(_rb(x - _rb(mean)) / den)


def _kernel(x_hbm, mem0_hbm, wq_hbm, wk_hbm, wv_hbm, wo_hbm, wr_hbm, wg_hbm, wu_hbm, wd_hbm,
            out_hbm,
            x_v, xn_v, mem_v, o_v, out_v, wq_v, wk_v, wv_v, wo_v, wg_v, wu_v, wd_v,
            rq_v, rk_v, rv_v, r_v, p_v, mq_v, mk_v, mv_v, h_v, xh_v, mem0_ref, wr_ref, sem_s,
            sem_x, sem_w, sem_o, sem_f, sem_out, sem_p,
            *, S, D, H, E, M, SEG, F, G, T, R0, RING, OFF):
    n_seg = S // SEG
    L = M + SEG
    NG = H // G
    NR = S // (8 * 128)
    scale = float(E) ** -0.5
    w_hbm = (wq_hbm, wk_hbm, wv_hbm)
    w_vm = (wq_v, wk_v, wv_v)
    ring = (rq_v, rk_v, rv_v)

    LNB = 128
    NP = R0 // LNB
    XH = R0 + 2 * SEG

    def x_copy(lo, hi, i):
        return pltpu.make_async_copy(x_hbm.at[pl.ds(lo, hi - lo)], x_v.at[pl.ds(lo, hi - lo)], sem_x.at[i])

    cp_x = [x_copy(i * LNB, (i + 1) * LNB, i) for i in range(NP)]
    cp_xm = x_copy(R0, XH, NP)
    cp_xt = x_copy(XH, S, NP + 1)
    cp_small = [pltpu.make_async_copy(mem0_hbm, mem0_ref, sem_s.at[0]),
                pltpu.make_async_copy(wr_hbm, wr_ref, sem_s.at[1])]

    def start_wo(c):
        rows = pl.ds(pl.multiple_of(c * (G * E // 2), 8), G * E // 2)
        pltpu.make_async_copy(wo_hbm.bitcast(I32).at[rows], wo_v.at[rows], sem_o).start()

    cp_f = [pltpu.make_async_copy(src.bitcast(I32), dst, sem_f.at[i])
            for i, (src, dst) in enumerate(((wg_hbm, wg_v), (wu_hbm, wu_v), (wd_hbm, wd_v)))]

    def start_w(m, g):
        for u in range(G):
            pltpu.make_async_copy(
                w_hbm[m].bitcast(I32).at[:, u % 2, g * (G // 2) + u // 2, :],
                w_vm[m].at[g * G + u], sem_w.at[m, g]).start()

    def wait_w(m, g):
        grp = pl.ds(pl.multiple_of(g * G, G), G)
        pltpu.make_async_copy(w_vm[m].at[grp], w_vm[m].at[grp], sem_w.at[m, g]).wait()

    def ln_rows(row0, n, packed=False):
        wr = wr_ref[...].astype(F32)
        xn = _layernorm(x_v[pl.ds(row0, n), :].astype(F32))
        xn_v[pl.ds(row0, n), :] = xn
        if packed:
            xh_v[pl.ds(pl.multiple_of(row0 // 2, n // 2), n // 2), :] = pltpu.bitcast(xn.astype(BF16), I32)
        acc = xn[:, 0:128] * wr[0:1, :]
        for j in range(1, D // 128):
            acc = acc + xn[:, j * 128:(j + 1) * 128] * wr[j:j + 1, :]
        r = jnp.broadcast_to(_rb(jnp.sum(acc, axis=-1, keepdims=True)), (n, 128))
        lane = lax.broadcasted_iota(I32, (8, 128), 1)
        for i in range(NR):
            slab = r_v[i]
            for t in range(n // 8):
                slab = jnp.where(lane == row0 // 8 + (t - 128 * i), r[t * 8:(t + 1) * 8], slab)
            r_v[i] = slab

    def project(m, g):
        ws = []
        for u in range(0, G, 2):
            a = w_vm[m][g * G + u]
            b = w_vm[m][g * G + u + 1]
            lo = (a & 0xFFFF) | (b << 16)
            hi = lax.shift_right_logical(a, 16) | (b & (-65536))
            w_vm[m][g * G + u] = lo
            w_vm[m][g * G + u + 1] = hi
            ws += [lo, hi]
        ring[m][g, pl.ds(OFF, R0), :] = _dot(_w(xh_v[...]), _w(jnp.concatenate(ws, axis=1)))

    for c in cp_x + cp_small:
        c.start()
    r_v[...] = jnp.full(r_v.shape, -jnp.inf, F32)
    for c in cp_small:
        c.wait()
    mem_v[...] = mem0_ref[...].astype(F32)
    for i in range(NP):
        cp_x[i].wait()
        if i == 0:
            start_w(0, 0)
        if i == 2:
            start_w(1, 0)
        ln_rows(i * LNB, LNB, packed=True)

    wait_w(0, 0)
    start_w(2, 0)
    project(0, 0)
    wait_w(1, 0)
    wait_w(2, 0)
    for m in range(3):
        start_w(m, 1)
    cp_xm.start()
    start_wo(0)
    project(1, 0)
    project(2, 0)

    def pro_body(g, c):
        for m in range(3):
            wait_w(m, g)

        @pl.when(g < NG - 1)
        def _():
            for m in range(3):
                start_w(m, g + 1)

        @pl.when(g == NG - 1)
        def _():
            cp_xt.start()

        start_wo(g)
        for m in range(3):
            project(m, g)
        return c

    lax.fori_loop(1, NG, pro_body, 0)
    cp_xm.wait()

    for c in cp_f:
        c.start()
    ln_rows(R0, T)
    cp_xt.wait()
    pltpu.make_async_copy(wo_v, wo_v, sem_o).wait()

    row = lax.broadcasted_iota(I32, (L, L), 0)
    col = lax.broadcasted_iota(I32, (L, L), 1)
    mask = (row < M) | (row >= col)
    hs = lambda u: slice(u * E, (u + 1) * E)

    def step(s, carry):
        row0 = pl.multiple_of(s * SEG, SEG)
        new0 = pl.multiple_of(R0 + s * T, 8)
        wr0 = pl.multiple_of(lax.rem(R0 + OFF + s * T, RING), 8)
        rd0 = pl.multiple_of(lax.rem(OFF + s * SEG, RING), SEG)

        mrow = (mq_v, mk_v, mv_v)
        h_v[...] = pltpu.bitcast(
            jnp.concatenate([mem_v[...], xn_v[pl.ds(new0, T), :]], axis=0).astype(BF16), I32)

        def proj(m, g):
            h = _w(h_v[...])
            w = jnp.concatenate([w_vm[m][g * G + u] for u in range(G)], axis=1)
            y = _dot(h, _w(w))
            ring[m][g, pl.ds(wr0, T), :] = y[M:]
            mrow[m][g % 2] = y[0:M]

        def seg_rows(m, g):
            return jnp.concatenate([mrow[m][g % 2], ring[m][g, pl.ds(rd0, SEG), :]], axis=0)

        def scores(g):
            q = seg_rows(0, g)
            k = seg_rows(1, g)
            for u in range(G):
                sc = jnp.where(mask, _dot(q[:, hs(u)], k[:, hs(u)], _NT), -1e9 / scale)
                e = jnp.exp2((sc - jnp.max(sc, axis=-1, keepdims=True)) * (scale * _LOG2E))
                p_v[g % 2, u] = e * _recip(jnp.sum(e, axis=-1, keepdims=True))

        def attend(g):
            v = seg_rows(2, g)
            for u in range(G):
                o_v[:, (g * G + u) * E:(g * G + u + 1) * E] = _dot(p_v[g % 2, u], v[:, hs(u)])

        def outproj(g0, g1):
            return _dot(o_v[:, g0 * G * E:g1 * G * E],
                        _w(wo_v[g0 * G * E // 2:g1 * G * E // 2, :]))

        for g in range(NG):
            proj(0, g)
            proj(1, g)
            if g > 0:
                attend(g - 1)
            proj(2, g)
            scores(g)
        y = outproj(0, NG - 2)
        attend(NG - 1)
        y = outproj(NG - 2, NG - 1) + y
        y = outproj(NG - 1, NG) + y
        mem_v[...] = y[0:M]
        res = (x_v[pl.ds(row0, SEG), :].astype(F32) + y[M:]) + xn_v[pl.ds(row0, SEG), :]
        out_v[pl.ds(row0, SEG), :] = res.astype(BF16)
        pltpu.make_async_copy(out_v.at[pl.ds(row0, SEG), :], out_hbm.at[pl.ds(row0, SEG), :],
                              sem_out).start()
        ln_rows(pl.multiple_of(jnp.minimum(new0 + T, S - T), 8), T)
        return carry

    def steps(i, c):
        for j in range(2):
            step(i * 2 + j, c)
        return c

    lax.fori_loop(0, n_seg // 2, steps, 0)

    pos = (lax.broadcasted_iota(I32, (8, 128), 1) * 8 + lax.broadcasted_iota(I32, (8, 128), 0))
    vals = [r_v[i] for i in range(NR)]
    toks = [(pos + 1024 * i).astype(F32) for i in range(NR)]

    def all_max(vs):
        m = functools.reduce(jnp.maximum, vs)
        return jnp.max(jnp.max(m, axis=0, keepdims=True), axis=1, keepdims=True)

    def first_with(vs, m):
        c = functools.reduce(jnp.minimum, [jnp.where(v == m, t, float(S)) for v, t in zip(vs, toks)])
        return jnp.min(jnp.min(c, axis=0, keepdims=True), axis=1, keepdims=True)

    m1 = all_max(vals)
    j1 = first_with(vals, m1)
    vals = [jnp.where(t == j1, -jnp.inf, v) for v, t in zip(vals, toks)]
    m2 = all_max(vals)
    j2 = first_with(vals, m2)
    j1 = j1.astype(I32)
    j2 = j2.astype(I32)
    t1 = jnp.clip(j1[0, 0], 0, S - 1)
    t2 = jnp.clip(j2[0, 0], 0, S - 1)

    sub = lax.broadcasted_iota(I32, (8, D), 0)
    xs = jnp.where(sub == 0, xn_v[pl.ds(t1, 1), :], xn_v[pl.ds(t2, 1), :])
    for c in cp_f:
        c.wait()
    gate = _dot(xs, _w(wg_v[...]))
    up = _dot(xs, _w(wu_v[...]))
    act = gate * jax.nn.sigmoid(gate) * up
    yf = _dot(act, _w(wd_v[...]))
    sub1 = lax.broadcasted_iota(I32, (8, 128), 0)
    rs = jax.nn.sigmoid(jnp.where(sub1 == 0, m1, m2))
    yf = yf * rs[:, 0:1]

    pltpu.make_async_copy(out_v, out_v, sem_out).wait()
    rows16 = lax.broadcasted_iota(I32, (16, D), 0)
    b1 = pl.multiple_of((t1 // 16) * 16, 16)
    b2 = pl.multiple_of((t2 // 16) * 16, 16)
    for b, t, i in ((b1, t1, 0), (b2, t2, 1)):
        blk = out_v[pl.ds(b, 16), :].astype(F32)
        out_v[pl.ds(b, 16), :] = jnp.where(rows16 == t - b, blk + yf[i:i + 1], blk).astype(BF16)
    cp1 = pltpu.make_async_copy(out_v.at[pl.ds(b1, 16), :], out_hbm.at[pl.ds(b1, 16), :], sem_p.at[0])
    cp1.start()

    @pl.when(b1 != b2)
    def _():
        cp2 = pltpu.make_async_copy(out_v.at[pl.ds(b2, 16), :], out_hbm.at[pl.ds(b2, 16), :],
                                    sem_p.at[1])
        cp2.start()
        cp2.wait()

    cp1.wait()


@functools.partial(jax.jit, static_argnames=("A_seg_len",))
def pallas_parallel_sum__memory_aug_recurrent_mem_tr__moe_arch_mod__prompt_kernel(
    A_x, A_mem0, A_Wq, A_Wk, A_Wv, A_Wo, A_seg_len, B_x, B_w_r, B_w_gate, B_w_up, B_w_down,
):
    del B_x
    B, S, D = A_x.shape
    _, H, E = A_Wq.shape
    M = A_mem0.shape[1]
    F = B_w_gate.shape[1]
    SEG = int(A_seg_len)
    assert B == 1
    L = M + SEG
    G = 4
    NG = H // G
    T = 24
    R0 = S - (S // SEG) * T
    RING, OFF = 576, 64
    assert (R0 + OFF) % T == 0 and OFF % SEG == 0 and RING % T == 0 and RING % SEG == 0
    assert R0 + OFF <= RING and R0 + T <= RING
    any_spec = pl.BlockSpec(memory_space=pl.ANY)
    vmem_spec = pl.BlockSpec(memory_space=pltpu.VMEM)
    kern = functools.partial(_kernel, S=S, D=D, H=H, E=E, M=M, SEG=SEG, F=F, G=G, T=T, R0=R0,
                             RING=RING, OFF=OFF)
    out = pl.pallas_call(
        kern,
        out_shape=jax.ShapeDtypeStruct((S, D), A_x.dtype),
        in_specs=[any_spec, any_spec, any_spec, any_spec, any_spec, any_spec, any_spec,
                  any_spec, any_spec, any_spec],
        out_specs=any_spec,
        scratch_shapes=[
            pltpu.VMEM((S, D), BF16),
            pltpu.VMEM((S, D), F32),
            pltpu.VMEM((M, D), F32),
            pltpu.VMEM((L, H * E), F32),
            pltpu.VMEM((S, D), BF16),
            pltpu.VMEM((H, D // 2, E), I32),
            pltpu.VMEM((H, D // 2, E), I32),
            pltpu.VMEM((H, D // 2, E), I32),
            pltpu.VMEM((H * E // 2, D), I32),
            pltpu.VMEM((D // 2, F), I32),
            pltpu.VMEM((D // 2, F), I32),
            pltpu.VMEM((F // 2, D), I32),
            pltpu.VMEM((NG, RING, G * E), F32),
            pltpu.VMEM((NG, RING, G * E), F32),
            pltpu.VMEM((NG, RING, G * E), F32),
            pltpu.VMEM((S // 1024, 8, 128), F32),
            pltpu.VMEM((2, G, L, L), F32),
            pltpu.VMEM((2, M, G * E), F32),
            pltpu.VMEM((2, M, G * E), F32),
            pltpu.VMEM((2, M, G * E), F32),
            pltpu.VMEM(((M + T) // 2, D), I32),
            pltpu.VMEM((R0 // 2, D), I32),
            pltpu.VMEM((M, D), BF16),
            pltpu.VMEM((D // 128, 128), BF16),
            pltpu.SemaphoreType.DMA((2,)),
            pltpu.SemaphoreType.DMA((R0 // 128 + 2,)),
            pltpu.SemaphoreType.DMA((3, NG)),
            pltpu.SemaphoreType.DMA(()),
            pltpu.SemaphoreType.DMA((3,)),
            pltpu.SemaphoreType.DMA(()),
            pltpu.SemaphoreType.DMA((2,)),
        ],
        compiler_params=pltpu.CompilerParams(vmem_limit_bytes=120 * 1024 * 1024),
    )(
        A_x.reshape(S, D), A_mem0.reshape(M, D),
        A_Wq.reshape(D // 2, 2, H, E), A_Wk.reshape(D // 2, 2, H, E), A_Wv.reshape(D // 2, 2, H, E),
        A_Wo.reshape(H * E, D), B_w_r.reshape(D // 128, 128), B_w_gate, B_w_up, B_w_down,
    )
    return out.reshape(B, S, D)
```

```python
import functools

import jax
import jax.numpy as jnp
import numpy as np
from jax import lax
import jax.experimental.pallas as pl
import jax.experimental.pallas.tpu as pltpu

CFG = {'prog': (('q', 0), ('L',), ('k', 0), ('v', 0), ('S', 0), ('q', 1), ('k', 1), ('A', 0), ('v', 1), ('S', 1), ('q', 2), ('k', 2), ('A', 1), ('v', 2), ('S', 2), ('q', 3), ('k', 3), ('A', 2), ('v', 3), ('S', 3), ('q', 4), ('k', 4), ('A', 3), ('v', 4), ('S', 4), ('q', 5), ('k', 5), ('A', 4), ('v', 5), ('S', 5), ('q', 6), ('k', 6), ('A', 5), ('v', 6), ('S', 6), ('q', 7), ('k', 7), ('A', 6), ('v', 7), ('S', 7), ('O', 0, 24), ('A', 7), ('O', 24, 28), ('O', 28, 32)), 'kbf': 1, 'vbf': 1, 'pmem': 1, 'hmem': 0, 'U': 2, 'dma_each': 1}

F32 = jnp.float32
BF16 = jnp.bfloat16
I32 = jnp.int32

_LOG2E = float(np.log2(np.e))
_NN = (((1,), (0,)), ((), ()))
_NT = (((1,), (1,)), ((), ()))


def _rb(x):
    return x.astype(BF16).astype(F32)


def _w(words):
    return pltpu.bitcast(words, BF16)


def _dot(a, b, dims=_NN):
    return lax.dot_general(a, b, dims, preferred_element_type=F32)


def _recip(x):
    r = pl.reciprocal(x, approx=True)
    return r * (2.0 - x * r)


def _layernorm(x):
    d = x.shape[-1]
    mean = jnp.sum(x, axis=-1, keepdims=True) * (1.0 / d)
    c = x - mean
    var = jnp.sum(c * c, axis=-1, keepdims=True) * (1.0 / d)
    eps = float(np.float32(np.asarray(1e-5, dtype=BF16)))
    den = _rb(jnp.sqrt(_rb(_rb(var) + eps)))
    return _rb(_rb(x - _rb(mean)) / den)


def _kernel(x_hbm, mem0_hbm, wq_hbm, wk_hbm, wv_hbm, wo_hbm, wr_hbm, wg_hbm, wu_hbm, wd_hbm,
            out_hbm,
            x_v, xn_v, mem_v, o_v, out_v, wq_v, wk_v, wv_v, wo_v, wg_v, wu_v, wd_v,
            rq_v, rk_v, rv_v, r_v, y_v, p_v, mq_v, mk_v, mv_v, h_v, xh_v, mem0_v, wr_v,
            sem_s, sem_x, sem_w, sem_o, sem_f, sem_out, sem_p,
            *, S, D, H, E, M, SEG, F, G, T, R0, RING, OFF):
    cfg = CFG.get
    n_seg = S // SEG
    L = M + SEG
    NG = H // G
    NR = S // (8 * 128)
    scale = float(E) ** -0.5
    w_hbm = (wq_hbm, wk_hbm, wv_hbm)
    w_vm = (wq_v, wk_v, wv_v)
    ring = (rq_v, rk_v, rv_v)
    mrow = (mq_v, mk_v, mv_v)

    LNB = 128
    NP = R0 // LNB
    XH = R0 + 2 * SEG

    def x_copy(lo, hi, i):
        return pltpu.make_async_copy(x_hbm.at[pl.ds(lo, hi - lo)], x_v.at[pl.ds(lo, hi - lo)],
                                     sem_x.at[i])

    cp_x = [x_copy(i * LNB, (i + 1) * LNB, i) for i in range(NP)]
    cp_xm = x_copy(R0, XH, NP)
    cp_xt = x_copy(XH, S, NP + 1)
    cp_small = [pltpu.make_async_copy(mem0_hbm, mem0_v, sem_s.at[0]),
                pltpu.make_async_copy(wr_hbm, wr_v, sem_s.at[1])]
    cp_f = [pltpu.make_async_copy(src.bitcast(I32), dst, sem_f.at[i])
            for i, (src, dst) in enumerate(((wg_hbm, wg_v), (wu_hbm, wu_v), (wd_hbm, wd_v)))]

    def start_wo(c):
        rows = pl.ds(pl.multiple_of(c * (G * E // 2), 8), G * E // 2)
        pltpu.make_async_copy(wo_hbm.bitcast(I32).at[rows], wo_v.at[rows], sem_o).start()

    def start_w(m, g):
        for u in range(G):
            pltpu.make_async_copy(
                w_hbm[m].bitcast(I32).at[:, u % 2, g * (G // 2) + u // 2, :],
                w_vm[m].at[g * G + u], sem_w.at[m, g]).start()

    def wait_w(m, g):
        grp = pl.ds(pl.multiple_of(g * G, G), G)
        pltpu.make_async_copy(w_vm[m].at[grp], w_vm[m].at[grp], sem_w.at[m, g]).wait()

    def ln_rows(row0, n, packed=False):
        wr = wr_v[...].astype(F32)
        xn = _layernorm(x_v[pl.ds(row0, n), :].astype(F32))
        xn_v[pl.ds(row0, n), :] = xn
        if packed:
            xh_v[pl.ds(row0 // 2, n // 2), :] = pltpu.bitcast(xn.astype(BF16), I32)
        acc = xn[:, 0:128] * wr[0:1, :]
        for j in range(1, D // 128):
            acc = acc + xn[:, j * 128:(j + 1) * 128] * wr[j:j + 1, :]
        r = jnp.broadcast_to(_rb(jnp.sum(acc, axis=-1, keepdims=True)), (n, 128))
        lane = lax.broadcasted_iota(I32, (8, 128), 1)
        for i in range(NR):
            slab = r_v[i]
            for t in range(n // 8):
                slab = jnp.where(lane == (row0 >> 3) + (t - 128 * i), r[t * 8:(t + 1) * 8], slab)
            r_v[i] = slab

    def project(m, g):
        ws = []
        for u in range(0, G, 2):
            a = w_vm[m][g * G + u]
            b = w_vm[m][g * G + u + 1]
            lo = (a & 0xFFFF) | (b << 16)
            hi = lax.shift_right_logical(a, 16) | (b & (-65536))
            w_vm[m][g * G + u] = lo
            w_vm[m][g * G + u + 1] = hi
            ws += [lo, hi]
        ring[m][g, pl.ds(OFF, R0), :] = _dot(_w(xh_v[...]), _w(jnp.concatenate(ws, axis=1)))

    for c in cp_x + cp_small:
        c.start()
    r_v[...] = jnp.full(r_v.shape, -jnp.inf, F32)
    for c in cp_small:
        c.wait()
    mem_v[...] = mem0_v[...].astype(F32)
    for i in range(NP):
        cp_x[i].wait()
        if i == 0:
            start_w(0, 0)
        if i == 2:
            start_w(1, 0)
        ln_rows(i * LNB, LNB, packed=True)

    wait_w(0, 0)
    start_w(2, 0)
    project(0, 0)
    wait_w(1, 0)
    wait_w(2, 0)
    for m in range(3):
        start_w(m, 1)
    cp_xm.start()
    start_wo(0)
    project(1, 0)
    project(2, 0)

    def pro_body(g, c):
        for m in range(3):
            wait_w(m, g)

        @pl.when(g < NG - 1)
        def _():
            for m in range(3):
                start_w(m, g + 1)

        @pl.when(g == NG - 1)
        def _():
            cp_xt.start()

        start_wo(g)
        for m in range(3):
            project(m, g)
        return c

    lax.fori_loop(1, NG, pro_body, 0)
    cp_xm.wait()
    for c in cp_f:
        c.start()
    ln_rows(R0, T)
    cp_xt.wait()
    pltpu.make_async_copy(wo_v, wo_v, sem_o).wait()

    hs = lambda u: slice(u * E, (u + 1) * E)

    def step(s, par):
        row = lax.broadcasted_iota(I32, (L, L), 0)
        col = lax.broadcasted_iota(I32, (L, L), 1)
        mask = (row < M) | (row >= col)
        row0 = pl.multiple_of(s * SEG, SEG)
        new0 = pl.multiple_of(R0 + s * T, 8)
        wr0 = pl.multiple_of(lax.rem(R0 + OFF + s * T, RING), 8)
        rd0 = pl.multiple_of(lax.rem(OFF + s * SEG, RING), SEG)
        hval = jnp.concatenate([mem_v[...], xn_v[pl.ds(new0, T), :]], axis=0).astype(BF16)
        if cfg("hmem", 1):
            h_v[par] = pltpu.bitcast(hval, I32)
        held = {}

        def keep(ref, key, val):
            if cfg("pmem" if key[0] == "p" else "mmem", 1):
                ref[key[1]] = val
            else:
                held[key] = val

        def fetch(ref, key):
            if cfg("pmem" if key[0] == "p" else "mmem", 1):
                return ref[key[1]]
            return held[key]

        def proj(m, g, u0=0, u1=G):
            h = _w(h_v[par]) if cfg("hmem", 1) else hval
            w = jnp.concatenate([w_vm[m][g * G + u] for u in range(u0, u1)], axis=1)
            y = _dot(h, _w(w))
            ring[m][g, pl.ds(wr0, T), u0 * E:u1 * E] = y[M:]
            for u in range(u0, u1):
                keep(mrow[m], (m, (g * G + u) % 16), y[0:M, hs(u - u0)])

        def seg_rows(m, g, u):
            return jnp.concatenate([fetch(mrow[m], (m, (g * G + u) % 16)),
                                    ring[m][g, pl.ds(rd0, SEG), hs(u)]], axis=0)

        def scores(g):
            for u in range(G):
                kk = seg_rows(1, g, u)
                if cfg("kbf", 0):
                    kk = kk.astype(BF16)
                sc = _dot(seg_rows(0, g, u), kk, _NT)
                if cfg("smx", 1) == 0:
                    sc = jnp.where(mask, sc * scale, -1e9)
                    e = jnp.exp(sc - jnp.max(sc, axis=-1, keepdims=True))
                    p = e / jnp.sum(e, axis=-1, keepdims=True)
                else:
                    sc = jnp.where(mask, sc, -1e9 / scale)
                    e = jnp.exp2((sc - jnp.max(sc, axis=-1, keepdims=True)) * (scale * _LOG2E))
                    p = e * _recip(jnp.sum(e, axis=-1, keepdims=True))
                keep(p_v, ("p", (g * G + u) % 16), p)

        def attend(g):
            for u in range(G):
                vv = seg_rows(2, g, u)
                if cfg("vbf", 0):
                    vv = vv.astype(BF16)
                o_v[:, (g * G + u) * E:(g * G + u + 1) * E] = _dot(
                    fetch(p_v, ("p", (g * G + u) % 16)), vv)

        state = {"y": None}

        def outproj(h0, h1):
            y = _dot(o_v[:, h0 * E:h1 * E], _w(wo_v[h0 * E // 2:h1 * E // 2, :]))
            if cfg("ymem", 0):
                if h0 > 0:
                    y = y + y_v[...]
                if h1 < H:
                    y_v[...] = y
            elif h0 > 0:
                y = y + state["y"]
            state["y"] = y

        def norm_next():
            ln_rows(pl.multiple_of(jnp.minimum(new0 + T, S - T), 8), T)

        for op in cfg("prog"):
            if op[0] in "qkv":
                proj("qkv".index(op[0]), *op[1:])
            elif op[0] == "S":
                scores(op[1])
            elif op[0] == "A":
                attend(op[1])
            elif op[0] == "O":
                outproj(op[1], op[2])
            elif op[0] == "L":
                norm_next()
        y = state["y"]
        mem_v[...] = y[0:M]
        res = (x_v[pl.ds(row0, SEG), :].astype(F32) + y[M:]) + xn_v[pl.ds(row0, SEG), :]
        out_v[pl.ds(row0, SEG), :] = res.astype(BF16)
        if cfg("dma_each", 1):
            pltpu.make_async_copy(out_v.at[pl.ds(row0, SEG), :], out_hbm.at[pl.ds(row0, SEG), :],
                                  sem_out).start()
        if ("L",) not in cfg("prog"):
            norm_next()

    U = cfg("U", 2)

    def steps(i, c):
        for j in range(U):
            step(i * U + j, j % 2)
        if not cfg("dma_each", 1):
            rows = pl.ds(pl.multiple_of(i * (U * SEG), U * SEG), U * SEG)
            pltpu.make_async_copy(out_v.at[rows, :], out_hbm.at[rows, :], sem_out).start()
        return c

    lax.fori_loop(0, n_seg // U, steps, 0)

    pos = (lax.broadcasted_iota(I32, (8, 128), 1) * 8 + lax.broadcasted_iota(I32, (8, 128), 0))
    vals = [r_v[i] for i in range(NR)]
    toks = [(pos + 1024 * i).astype(F32) for i in range(NR)]

    def all_max(vs):
        m = functools.reduce(jnp.maximum, vs)
        return jnp.max(jnp.max(m, axis=0, keepdims=True), axis=1, keepdims=True)

    def first_with(vs, m):
        c = functools.reduce(jnp.minimum,
                             [jnp.where(v == m, t, float(S)) for v, t in zip(vs, toks)])
        return jnp.min(jnp.min(c, axis=0, keepdims=True), axis=1, keepdims=True)

    m1 = all_max(vals)
    j1 = first_with(vals, m1)
    vals = [jnp.where(t == j1, -jnp.inf, v) for v, t in zip(vals, toks)]
    m2 = all_max(vals)
    j2 = first_with(vals, m2)
    t1 = jnp.clip(j1.astype(I32)[0, 0], 0, S - 1)
    t2 = jnp.clip(j2.astype(I32)[0, 0], 0, S - 1)

    sub = lax.broadcasted_iota(I32, (8, D), 0)
    xs = jnp.where(sub == 0, xn_v[pl.ds(t1, 1), :], xn_v[pl.ds(t2, 1), :])
    for c in cp_f:
        c.wait()
    gate = _dot(xs, _w(wg_v[...]))
    up = _dot(xs, _w(wu_v[...]))
    act = gate * jax.nn.sigmoid(gate) * up
    yf = _dot(act, _w(wd_v[...]))
    sub1 = lax.broadcasted_iota(I32, (8, 128), 0)
    rs = jax.nn.sigmoid(jnp.where(sub1 == 0, m1, m2))
    yf = yf * rs[:, 0:1]

    pltpu.make_async_copy(out_v, out_v, sem_out).wait()
    rows16 = lax.broadcasted_iota(I32, (16, D), 0)
    b1 = pl.multiple_of((t1 >> 4) << 4, 16)
    b2 = pl.multiple_of((t2 >> 4) << 4, 16)
    for b, t, i in ((b1, t1, 0), (b2, t2, 1)):
        blk = out_v[pl.ds(b, 16), :].astype(F32)
        out_v[pl.ds(b, 16), :] = jnp.where(rows16 == t - b, blk + yf[i:i + 1], blk).astype(BF16)
    cp1 = pltpu.make_async_copy(out_v.at[pl.ds(b1, 16), :], out_hbm.at[pl.ds(b1, 16), :],
                                sem_p.at[0])
    cp1.start()

    @pl.when(b1 != b2)
    def _():
        cp2 = pltpu.make_async_copy(out_v.at[pl.ds(b2, 16), :], out_hbm.at[pl.ds(b2, 16), :],
                                    sem_p.at[1])
        cp2.start()
        cp2.wait()

    cp1.wait()


@functools.partial(jax.jit, static_argnames=("A_seg_len",))
def pallas_parallel_sum__memory_aug_recurrent_mem_tr__moe_arch_mod__prompt_kernel(
    A_x, A_mem0, A_Wq, A_Wk, A_Wv, A_Wo, A_seg_len, B_x, B_w_r, B_w_gate, B_w_up, B_w_down,
):
    del B_x
    B, S, D = A_x.shape
    _, H, E = A_Wq.shape
    M = A_mem0.shape[1]
    F = B_w_gate.shape[1]
    SEG = int(A_seg_len)
    assert B == 1
    L = M + SEG
    G = 4
    NG = H // G
    T = 24
    R0 = S - (S // SEG) * T
    RING, OFF = 576, 64
    assert (R0 + OFF) % T == 0 and OFF % SEG == 0 and RING % T == 0 and RING % SEG == 0
    assert R0 + OFF <= RING and R0 + T <= RING
    any_spec = pl.BlockSpec(memory_space=pl.ANY)
    kern = functools.partial(_kernel, S=S, D=D, H=H, E=E, M=M, SEG=SEG, F=F, G=G, T=T, R0=R0,
                             RING=RING, OFF=OFF)
    out = pl.pallas_call(
        kern,
        out_shape=jax.ShapeDtypeStruct((S, D), A_x.dtype),
        in_specs=[any_spec] * 10,
        out_specs=any_spec,
        scratch_shapes=[
            pltpu.VMEM((S, D), BF16),
            pltpu.VMEM((S, D), F32),
            pltpu.VMEM((M, D), F32),
            pltpu.VMEM((L, H * E), F32),
            pltpu.VMEM((S, D), BF16),
            pltpu.VMEM((H, D // 2, E), I32),
            pltpu.VMEM((H, D // 2, E), I32),
            pltpu.VMEM((H, D // 2, E), I32),
            pltpu.VMEM((H * E // 2, D), I32),
            pltpu.VMEM((D // 2, F), I32),
            pltpu.VMEM((D // 2, F), I32),
            pltpu.VMEM((F // 2, D), I32),
            pltpu.VMEM((NG, RING, G * E), F32),
            pltpu.VMEM((NG, RING, G * E), F32),
            pltpu.VMEM((NG, RING, G * E), F32),
            pltpu.VMEM((S // 1024, 8, 128), F32),
            pltpu.VMEM((L, D), F32),
            pltpu.VMEM((16, L, L), F32),
            pltpu.VMEM((16, M, E), F32),
            pltpu.VMEM((16, M, E), F32),
            pltpu.VMEM((16, M, E), F32),
            pltpu.VMEM((2, (M + T) // 2, D), I32),
            pltpu.VMEM((R0 // 2, D), I32),
            pltpu.VMEM((M, D), BF16),
            pltpu.VMEM((D // 128, 128), BF16),
            pltpu.SemaphoreType.DMA((2,)),
            pltpu.SemaphoreType.DMA((R0 // 128 + 2,)),
            pltpu.SemaphoreType.DMA((3, NG)),
            pltpu.SemaphoreType.DMA(()),
            pltpu.SemaphoreType.DMA((3,)),
            pltpu.SemaphoreType.DMA(()),
            pltpu.SemaphoreType.DMA((2,)),
        ],
        compiler_params=pltpu.CompilerParams(vmem_limit_bytes=120 * 1024 * 1024,
                                             flags=CFG.get("flags")),
    )(
        A_x.reshape(S, D), A_mem0.reshape(M, D),
        A_Wq.reshape(D // 2, 2, H, E), A_Wk.reshape(D // 2, 2, H, E), A_Wv.reshape(D // 2, 2, H, E),
        A_Wo.reshape(H * E, D), B_w_r.reshape(D // 128, 128), B_w_gate, B_w_up, B_w_down,
    )
    return out.reshape(B, S, D)
```

```python
import functools

import jax
import jax.numpy as jnp
import numpy as np
from jax import lax
import jax.experimental.pallas as pl
import jax.experimental.pallas.tpu as pltpu

F32 = jnp.float32
BF16 = jnp.bfloat16
I32 = jnp.int32

_LOG2E = float(np.log2(np.e))
_NN = (((1,), (0,)), ((), ()))
_NT = (((1,), (1,)), ((), ()))

G = 4
T = 24
LN_HEAD = 128
LN_STEP = 32
FC = 256
UNROLL = 2


def _rb(x):
    return x.astype(BF16).astype(F32)


def _unpack(words):
    return pltpu.bitcast(words, BF16)


def _dot(a, b, dims=_NN):
    return lax.dot_general(a, b, dims, preferred_element_type=F32)


def _recip(x):
    r = pl.reciprocal(x, approx=True)
    return r * (2.0 - x * r)


def _layernorm(x):
    d = x.shape[-1]
    mean = jnp.sum(x, axis=-1, keepdims=True) * (1.0 / d)
    c = x - mean
    var = jnp.sum(c * c, axis=-1, keepdims=True) * (1.0 / d)
    eps = float(np.asarray(1e-5, dtype=BF16).astype(np.float32))
    den = _rb(jnp.sqrt(_rb(_rb(var) + eps)))
    return _rb(_rb(x - _rb(mean)) / den)


def _kernel(x_hbm, mem0_hbm, wq_hbm, wk_hbm, wv_hbm, wo_hbm, wr_hbm, wg_hbm, wu_hbm, wd_hbm,
            out_hbm,
            x_v, xn_v, xh_v, out_v, mem0_v, wr_v, mem_v, o_v, p_v, mq_v, mk_v, mv_v,
            wq_v, wk_v, wv_v, wo_v, wg_v, wu_v, wd_v, rq_v, rk_v, rv_v, r_v, xs_v, yf_v,
            sem_s, sem_x, sem_w, sem_o, sem_f, sem_out, sem_p,
            *, seg, r0, off):
    S, D = x_v.shape
    H, _, E = wq_v.shape
    M = mem_v.shape[0]
    F = wg_v.shape[1]
    ring_rows = rq_v.shape[1]
    n_seg = S // seg
    n_grp = H // G
    n_ffn = F // FC
    L = M + seg
    HD = D // 2
    scale = float(E) ** -0.5
    w_hbm = (wq_hbm, wk_hbm, wv_hbm)
    w_vm = (wq_v, wk_v, wv_v)
    ring = (rq_v, rk_v, rv_v)
    mem_rows = (mq_v, mk_v, mv_v)

    def x_copy(lo, hi, i):
        rows = pl.ds(lo, hi - lo)
        return pltpu.make_async_copy(x_hbm.at[rows], x_v.at[rows], sem_x.at[i])

    n_head = r0 // LN_HEAD
    cp_x = [x_copy(i * LN_HEAD, (i + 1) * LN_HEAD, i) for i in range(n_head)]
    cp_x_mid = x_copy(r0, r0 + 2 * seg, n_head)
    cp_x_tail = x_copy(r0 + 2 * seg, S, n_head + 1)
    cp_small = [pltpu.make_async_copy(mem0_hbm, mem0_v, sem_s.at[0]),
                pltpu.make_async_copy(wr_hbm, wr_v, sem_s.at[1])]
    cp_ffn = [pltpu.make_async_copy(src.bitcast(I32), dst, sem_f.at[i])
              for i, (src, dst) in enumerate(((wg_hbm, wg_v), (wu_hbm, wu_v), (wd_hbm, wd_v)))]

    def start_wo(g):
        rows = pl.ds(pl.multiple_of(g * (G * E // 2), 8), G * E // 2)
        pltpu.make_async_copy(wo_hbm.bitcast(I32).at[rows], wo_v.at[rows], sem_o).start()

    def start_w(m, g, priority=0):
        for u in range(G):
            pltpu.make_async_copy(
                w_hbm[m].bitcast(I32).at[:, u % 2, g * (G // 2) + u // 2, :],
                w_vm[m].at[g * G + u], sem_w.at[m, g]).start(priority=priority)

    def wait_w(m, g):
        grp = w_vm[m].at[pl.ds(pl.multiple_of(g * G, G), G)]
        pltpu.make_async_copy(grp, grp, sem_w.at[m, g]).wait()

    def out_copy(row0, n, sem):
        return pltpu.make_async_copy(out_v.at[pl.ds(row0, n), :], out_hbm.at[pl.ds(row0, n), :],
                                     sem)

    def normalise(row0, n, packed=False):
        wr = wr_v[...].astype(F32)
        xn = _layernorm(x_v[pl.ds(row0, n), :].astype(F32))
        xn_v[pl.ds(row0, n), :] = xn
        if packed:
            xh_v[pl.ds(row0 // 2, n // 2), :] = pltpu.bitcast(xn.astype(BF16), I32)
        acc = xn[:, 0:128] * wr[0:1, :]
        for j in range(1, D // 128):
            acc = acc + xn[:, j * 128:(j + 1) * 128] * wr[j:j + 1, :]
        r = jnp.broadcast_to(_rb(jnp.sum(acc, axis=-1, keepdims=True)), (n, 128))
        lane = lax.broadcasted_iota(I32, (8, 128), 1)
        for i in range(r_v.shape[0]):
            slab = r_v[i]
            for t in range(n // 8):
                slab = jnp.where(lane == (row0 >> 3) + (t - 128 * i), r[t * 8:(t + 1) * 8], slab)
            r_v[i] = slab

    def project_head(m, g):
        ws = []
        for u in range(0, G, 2):
            even = w_vm[m][g * G + u]
            odd = w_vm[m][g * G + u + 1]
            lo = (even & 0xFFFF) | (odd << 16)
            hi = lax.shift_right_logical(even, 16) | (odd & (-65536))
            w_vm[m][g * G + u] = lo
            w_vm[m][g * G + u + 1] = hi
            ws += [lo, hi]
        ring[m][g, pl.ds(off, r0), :] = _dot(_unpack(xh_v[...]),
                                             _unpack(jnp.concatenate(ws, axis=1)))

    cp_x[0].start()
    cp_x[1].start()
    start_w(0, 0, priority=1)
    for c in cp_small:
        c.start()
    r_v[...] = jnp.full(r_v.shape, -jnp.inf, F32)
    for c in cp_small:
        c.wait()
    mem_v[...] = mem0_v[...].astype(F32)
    for i in range(n_head):
        cp_x[i].wait()
        if i == 0:
            for c in cp_x[2:]:
                c.start()
        if i == 2:
            start_w(1, 0, priority=1)
        normalise(i * LN_HEAD, LN_HEAD, packed=True)

    wait_w(0, 0)
    start_w(2, 0)
    project_head(0, 0)
    wait_w(1, 0)
    wait_w(2, 0)
    for m in range(3):
        start_w(m, 1)
    cp_x_mid.start()
    start_wo(0)
    project_head(1, 0)
    project_head(2, 0)

    def prologue_body(g, carry):
        for m in range(3):
            wait_w(m, g)

        @pl.when(g < n_grp - 1)
        def _():
            for m in range(3):
                start_w(m, g + 1)

        @pl.when(g == n_grp - 1)
        def _():
            cp_x_tail.start()

        start_wo(g)
        for m in range(3):
            project_head(m, g)
        return carry

    lax.fori_loop(1, n_grp, prologue_body, 0)
    cp_x_mid.wait()
    for c in cp_ffn:
        c.start()
    normalise(r0, T)
    cp_x_tail.wait()
    pltpu.make_async_copy(wo_v, wo_v, sem_o).wait()

    def head_cols(u):
        return slice(u * E, (u + 1) * E)

    def step(s, ffn_chunk=None):
        row = lax.broadcasted_iota(I32, (L, L), 0)
        col = lax.broadcasted_iota(I32, (L, L), 1)
        mask = (row < M) | (row >= col)
        row0 = pl.multiple_of(s * seg, seg)
        new0 = pl.multiple_of(r0 + s * T, 8)
        ring_wr = pl.multiple_of(lax.rem(r0 + off + s * T, ring_rows), 8)
        ring_rd = pl.multiple_of(lax.rem(off + s * seg, ring_rows), seg)
        h = jnp.concatenate([mem_v[...], xn_v[pl.ds(new0, T), :]], axis=0).astype(BF16)

        def slot(g, u):
            return (g * G + u) % p_v.shape[0]

        def project(m, g):
            w = jnp.concatenate([w_vm[m][g * G + u] for u in range(G)], axis=1)
            y = _dot(h, _unpack(w))
            ring[m][g, pl.ds(ring_wr, T), :] = y[M:]
            for u in range(G):
                mem_rows[m][slot(g, u)] = y[0:M, head_cols(u)]

        def segment(m, g, u):
            return jnp.concatenate(
                [mem_rows[m][slot(g, u)], ring[m][g, pl.ds(ring_rd, seg), head_cols(u)]], axis=0)

        def probabilities(g):
            for u in range(G):
                sc = jnp.where(mask, _dot(segment(0, g, u), segment(1, g, u), _NT), -1e9 / scale)
                e = jnp.exp2((sc - jnp.max(sc, axis=-1, keepdims=True)) * (scale * _LOG2E))
                p_v[slot(g, u)] = e * _recip(jnp.sum(e, axis=-1, keepdims=True))

        def attend(g):
            for u in range(G):
                o_v[:, head_cols(g * G + u)] = _dot(p_v[slot(g, u)],
                                                    segment(2, g, u).astype(BF16))

        ys = [None, None]

        def project_out(g, half):
            w = wo_v[g * G * E // 2:(g + 1) * G * E // 2, half * HD:(half + 1) * HD]
            y = _dot(o_v[:, g * G * E:(g + 1) * G * E], _unpack(w))
            ys[half] = y if ys[half] is None else y + ys[half]

        ffn = {}

        def ffn_up(j):
            cols = pl.ds(pl.multiple_of(ffn_chunk * FC, 128), FC)
            rows = slice(j * 64, (j + 1) * 64)
            w = jnp.concatenate([wg_v[rows, cols], wu_v[rows, cols]], axis=1)
            t = _dot(xs_v[:, j * 128:(j + 1) * 128], _unpack(w))
            ffn["pre"] = t if j == 0 else t + ffn["pre"]

        def ffn_down(j):
            if "act" not in ffn:
                gate, up = ffn["pre"][:, :FC], ffn["pre"][:, FC:]
                ffn["act"] = gate * jax.nn.sigmoid(gate) * up
            kb, half = j % (FC // 128), j // (FC // 128)
            rows = pl.ds(pl.multiple_of(ffn_chunk * (FC // 2) + kb * 64, 64), 64)
            cols = slice(half * HD, (half + 1) * HD)
            yf_v[:, cols] = (_dot(ffn["act"][:, kb * 128:(kb + 1) * 128], _unpack(wd_v[rows, cols]))
                             + yf_v[:, cols])

        for g in range(n_grp):
            project(0, g)
            project(1, g)
            if ffn_chunk is None and g == n_grp - 3:
                normalise(pl.multiple_of(jnp.minimum(r0 + T + s * LN_STEP, S - LN_STEP), 8),
                          LN_STEP)
            if g > 0:
                attend(g - 1)
            project(2, g)
            probabilities(g)
        early = [(g, half) for half in range(2) for g in range(n_grp - 2)]
        late = [(g, half) for g in range(n_grp - 2, n_grp) for half in range(2)]
        n_up, n_down = D // 128, 2 * FC // 128
        for i, (g, half) in enumerate(early + late):
            if i == len(early):
                attend(n_grp - 1)
            project_out(g, half)
            if ffn_chunk is not None:
                if i < n_up:
                    ffn_up(i)
                if 0 <= i - (len(early) - 1) < n_down:
                    ffn_down(i - (len(early) - 1))

        y = jnp.concatenate(ys, axis=1)
        mem_v[...] = y[0:M]
        res = (x_v[pl.ds(row0, seg), :].astype(F32) + y[M:]) + xn_v[pl.ds(row0, seg), :]
        out_v[pl.ds(row0, seg), :] = res.astype(BF16)
        return out_copy(row0, seg, sem_out)

    def plain_steps(i, carry):
        for j in range(UNROLL):
            step(i * UNROLL + j).start()
        return carry

    lax.fori_loop(0, (n_seg - n_ffn) // UNROLL, plain_steps, 0)

    pos = lax.broadcasted_iota(I32, (8, 128), 1) * 8 + lax.broadcasted_iota(I32, (8, 128), 0)
    vals = [r_v[i] for i in range(r_v.shape[0])]
    toks = [(pos + 1024 * i).astype(F32) for i in range(r_v.shape[0])]

    def largest(vs):
        m = functools.reduce(jnp.maximum, vs)
        return jnp.max(jnp.max(m, axis=0, keepdims=True), axis=1, keepdims=True)

    def first_with(vs, m):
        c = functools.reduce(jnp.minimum,
                             [jnp.where(v == m, t, float(S)) for v, t in zip(vs, toks)])
        return jnp.min(jnp.min(c, axis=0, keepdims=True), axis=1, keepdims=True)

    m1 = largest(vals)
    j1 = first_with(vals, m1)
    vals = [jnp.where(t == j1, -jnp.inf, v) for v, t in zip(vals, toks)]
    m2 = largest(vals)
    j2 = first_with(vals, m2)
    t1 = jnp.clip(j1.astype(I32)[0, 0], 0, S - 1)
    t2 = jnp.clip(j2.astype(I32)[0, 0], 0, S - 1)

    first_row = lax.broadcasted_iota(I32, (8, D), 0) == 0
    xs_v[...] = jnp.where(first_row, xn_v[pl.ds(t1, 1), :], xn_v[pl.ds(t2, 1), :])
    yf_v[...] = jnp.zeros(yf_v.shape, F32)
    for c in cp_ffn:
        c.wait()

    def ffn_steps(i, carry):
        for j in range(UNROLL):
            copy = step(n_seg - n_ffn + i * UNROLL + j, i * UNROLL + j)
            if j < UNROLL - 1:
                copy.start()
            else:
                pl.when(i < n_ffn // UNROLL - 1)(copy.start)
        return carry

    lax.fori_loop(0, n_ffn // UNROLL, ffn_steps, 0)

    gate = jax.nn.sigmoid(jnp.where(lax.broadcasted_iota(I32, (8, 128), 0) == 0, m1, m2))
    yf = yf_v[...] * gate[:, 0:1]
    sent = out_v.at[pl.ds(0, S - seg), :]
    pltpu.make_async_copy(sent, sent, sem_out).wait()
    rows16 = lax.broadcasted_iota(I32, (16, D), 0)
    b1 = pl.multiple_of((t1 >> 4) << 4, 16)
    b2 = pl.multiple_of((t2 >> 4) << 4, 16)
    for b, t, i in ((b1, t1, 0), (b2, t2, 1)):
        blk = out_v[pl.ds(b, 16), :].astype(F32)
        out_v[pl.ds(b, 16), :] = jnp.where(rows16 == t - b, blk + yf[i:i + 1], blk).astype(BF16)

    last = out_copy(S - seg, seg, sem_out)
    last.start()
    resend = [(b1 < S - seg, out_copy(b1, 16, sem_p.at[0])),
              ((b2 < S - seg) & (b2 != b1), out_copy(b2, 16, sem_p.at[1]))]
    for cond, copy in resend:
        pl.when(cond)(copy.start)
    for cond, copy in resend:
        pl.when(cond)(copy.wait)
    last.wait()


@functools.partial(jax.jit, static_argnames=("A_seg_len",))
def pallas_parallel_sum__memory_aug_recurrent_mem_tr__moe_arch_mod__prompt_kernel(
    A_x, A_mem0, A_Wq, A_Wk, A_Wv, A_Wo, A_seg_len, B_x, B_w_r, B_w_gate, B_w_up, B_w_down,
):
    del B_x
    B, S, D = A_x.shape
    _, H, E = A_Wq.shape
    M = A_mem0.shape[1]
    F = B_w_gate.shape[1]
    seg = int(A_seg_len)
    L = M + seg
    n_seg, n_grp, n_ffn = S // seg, H // G, F // FC
    r0 = S - n_seg * T
    ring_rows, off = 576, 64
    assert B == 1 and S % seg == 0 and S % 1024 == 0 and E == 128 and F % FC == 0
    assert (r0 + off) % T == 0 and off % seg == 0 and ring_rows % T == 0 and ring_rows % seg == 0
    assert r0 + off <= ring_rows and r0 + T <= ring_rows and seg - T <= r0 // (n_seg - 1)
    assert r0 % LN_HEAD == 0 and r0 // LN_HEAD >= 3 and T <= 2 * seg and T <= LN_STEP
    assert r0 + T + (n_seg - n_ffn) * LN_STEP >= S
    assert n_ffn % UNROLL == 0 and n_seg % UNROLL == 0

    any_spec = pl.BlockSpec(memory_space=pl.ANY)
    out = pl.pallas_call(
        functools.partial(_kernel, seg=seg, r0=r0, off=off),
        out_shape=jax.ShapeDtypeStruct((S, D), A_x.dtype),
        in_specs=[any_spec] * 10,
        out_specs=any_spec,
        scratch_shapes=[
            pltpu.VMEM((S, D), BF16),
            pltpu.VMEM((S, D), F32),
            pltpu.VMEM((r0 // 2, D), I32),
            pltpu.VMEM((S, D), BF16),
            pltpu.VMEM((M, D), BF16),
            pltpu.VMEM((D // 128, 128), BF16),
            pltpu.VMEM((M, D), F32),
            pltpu.VMEM((L, H * E), F32),
            pltpu.VMEM((4 * G, L, L), F32),
            pltpu.VMEM((4 * G, M, E), F32),
            pltpu.VMEM((4 * G, M, E), F32),
            pltpu.VMEM((4 * G, M, E), F32),
            pltpu.VMEM((H, D // 2, E), I32),
            pltpu.VMEM((H, D // 2, E), I32),
            pltpu.VMEM((H, D // 2, E), I32),
            pltpu.VMEM((H * E // 2, D), I32),
            pltpu.VMEM((D // 2, F), I32),
            pltpu.VMEM((D // 2, F), I32),
            pltpu.VMEM((F // 2, D), I32),
            pltpu.VMEM((n_grp, ring_rows, G * E), F32),
            pltpu.VMEM((n_grp, ring_rows, G * E), F32),
            pltpu.VMEM((n_grp, ring_rows, G * E), F32),
            pltpu.VMEM((S // 1024, 8, 128), F32),
            pltpu.VMEM((8, D), F32),
            pltpu.VMEM((8, D), F32),
            pltpu.SemaphoreType.DMA((2,)),
            pltpu.SemaphoreType.DMA((r0 // LN_HEAD + 2,)),
            pltpu.SemaphoreType.DMA((3, n_grp)),
            pltpu.SemaphoreType.DMA(()),
            pltpu.SemaphoreType.DMA((3,)),
            pltpu.SemaphoreType.DMA(()),
            pltpu.SemaphoreType.DMA((2,)),
        ],
        compiler_params=pltpu.CompilerParams(vmem_limit_bytes=120 * 1024 * 1024),
    )(
        A_x.reshape(S, D), A_mem0.reshape(M, D),
        A_Wq.reshape(D // 2, 2, H, E), A_Wk.reshape(D // 2, 2, H, E), A_Wv.reshape(D // 2, 2, H, E),
        A_Wo.reshape(H * E, D), B_w_r.reshape(D // 128, 128), B_w_gate, B_w_up, B_w_down,
    )
    return out.reshape(B, S, D)
```

```python
import functools

import jax
import jax.numpy as jnp
import numpy as np
from jax import lax
import jax.experimental.pallas as pl
import jax.experimental.pallas.tpu as pltpu

F32 = jnp.float32
BF16 = jnp.bfloat16
I32 = jnp.int32

_LOG2E = float(np.log2(np.e))
_NN = (((1,), (0,)), ((), ()))
_NT = (((1,), (1,)), ((), ()))

G = 4
T = 24
LN_HEAD = 128
LN_STEP = 32
FC = 256
UNROLL = 2


def _rb(x):
    return x.astype(BF16).astype(F32)


def _unpack(words):
    return pltpu.bitcast(words, BF16)


def _dot(a, b, dims=_NN):
    return lax.dot_general(a, b, dims, preferred_element_type=F32)


def _recip(x):
    r = pl.reciprocal(x, approx=True)
    return r * (2.0 - x * r)


def _layernorm(x):
    d = x.shape[-1]
    mean = jnp.sum(x, axis=-1, keepdims=True) * (1.0 / d)
    c = x - mean
    var = jnp.sum(c * c, axis=-1, keepdims=True) * (1.0 / d)
    eps = float(np.asarray(1e-5, dtype=BF16).astype(np.float32))
    den = _rb(jnp.sqrt(_rb(_rb(var) + eps)))
    return _rb(_rb(x - _rb(mean)) / den)


def _kernel(x_hbm, mem0_hbm, wq_hbm, wk_hbm, wv_hbm, wo_hbm, wr_hbm, wg_hbm, wu_hbm, wd_hbm,
            out_hbm,
            x_v, xn_v, xh_v, out_v, mem0_v, wr_v, mem_v, o_v, p_v, mq_v, mk_v, mv_v,
            wq_v, wk_v, wv_v, wo_v, wg_v, wu_v, wd_v, rq_v, rk_v, rv_v, r_v, xs_v, yf_v, top_v,
            sem_s, sem_x, sem_w, sem_o, sem_f, sem_out, sem_p,
            *, seg, r0, off):
    S, D = x_v.shape
    H, _, E = wq_v.shape
    M = mem_v.shape[0]
    F = wg_v.shape[1]
    ring_rows = rq_v.shape[1]
    n_seg = S // seg
    n_grp = H // G
    n_ffn = F // FC
    L = M + seg
    HD = D // 2
    scale = float(E) ** -0.5
    w_hbm = (wq_hbm, wk_hbm, wv_hbm)
    w_vm = (wq_v, wk_v, wv_v)
    ring = (rq_v, rk_v, rv_v)
    mem_rows = (mq_v, mk_v, mv_v)

    def x_copy(lo, hi, i):
        rows = pl.ds(lo, hi - lo)
        return pltpu.make_async_copy(x_hbm.at[rows], x_v.at[rows], sem_x.at[i])

    n_head = r0 // LN_HEAD
    edges = [i * LN_HEAD for i in range(n_head)] + [r0 + seg, S]
    cp_x = [x_copy(edges[i], edges[i + 1], i) for i in range(n_head)]
    cp_x_tail = x_copy(edges[n_head], S, n_head)
    cp_small = [pltpu.make_async_copy(mem0_hbm, mem0_v, sem_s.at[0]),
                pltpu.make_async_copy(wr_hbm, wr_v, sem_s.at[1])]
    cp_ffn = [pltpu.make_async_copy(src.bitcast(I32), dst, sem_f.at[i])
              for i, (src, dst) in enumerate(((wg_hbm, wg_v), (wu_hbm, wu_v), (wd_hbm, wd_v)))]

    def start_wo(g):
        rows = pl.ds(pl.multiple_of(g * (G * E // 2), 8), G * E // 2)
        pltpu.make_async_copy(wo_hbm.bitcast(I32).at[rows], wo_v.at[rows], sem_o).start()

    def start_w(m, g, priority=0):
        for u in range(G):
            pltpu.make_async_copy(
                w_hbm[m].bitcast(I32).at[:, u % 2, g * (G // 2) + u // 2, :],
                w_vm[m].at[g * G + u], sem_w.at[m, g]).start(priority=priority)

    def wait_w(m, g):
        grp = w_vm[m].at[pl.ds(pl.multiple_of(g * G, G), G)]
        pltpu.make_async_copy(grp, grp, sem_w.at[m, g]).wait()

    def out_copy(row0, n, sem):
        return pltpu.make_async_copy(out_v.at[pl.ds(row0, n), :], out_hbm.at[pl.ds(row0, n), :],
                                     sem)

    def normalise(row0, n, packed=False):
        wr = wr_v[...].astype(F32)
        xn = _layernorm(x_v[pl.ds(row0, n), :].astype(F32))
        xn_v[pl.ds(row0, n), :] = xn
        if packed:
            xh_v[pl.ds(row0 // 2, n // 2), :] = pltpu.bitcast(xn.astype(BF16), I32)
        acc = xn[:, 0:128] * wr[0:1, :]
        for j in range(1, D // 128):
            acc = acc + xn[:, j * 128:(j + 1) * 128] * wr[j:j + 1, :]
        r = jnp.broadcast_to(_rb(jnp.sum(acc, axis=-1, keepdims=True)), (n, 128))
        lane = lax.broadcasted_iota(I32, (8, 128), 1)
        for i in range(r_v.shape[0]):
            slab = r_v[i]
            for t in range(n // 8):
                slab = jnp.where(lane == (row0 >> 3) + (t - 128 * i), r[t * 8:(t + 1) * 8], slab)
            r_v[i] = slab

    def project_head(m, g):
        ws = []
        for u in range(0, G, 2):
            even = w_vm[m][g * G + u]
            odd = w_vm[m][g * G + u + 1]
            lo = (even & 0xFFFF) | (odd << 16)
            hi = lax.shift_right_logical(even, 16) | (odd & (-65536))
            w_vm[m][g * G + u] = lo
            w_vm[m][g * G + u + 1] = hi
            ws += [lo, hi]
        ring[m][g, pl.ds(off, r0), :] = _dot(_unpack(xh_v[...]),
                                             _unpack(jnp.concatenate(ws, axis=1)))

    cp_x[0].start()
    cp_x[1].start()
    start_w(0, 0, priority=1)
    for c in cp_small:
        c.start()
    r_v[...] = jnp.full(r_v.shape, -jnp.inf, F32)
    for c in cp_small:
        c.wait()
    mem_v[...] = mem0_v[...].astype(F32)
    for i in range(n_head):
        cp_x[i].wait()
        if i == 0:
            for c in cp_x[2:]:
                c.start()
        if i == 2:
            start_w(1, 0, priority=1)
        normalise(i * LN_HEAD, LN_HEAD, packed=True)

    wait_w(0, 0)
    start_w(2, 0)
    project_head(0, 0)
    wait_w(1, 0)
    wait_w(2, 0)
    for m in range(3):
        start_w(m, 1)
    start_wo(0)
    project_head(1, 0)
    normalise(r0, T)
    project_head(2, 0)

    def prologue_body(g, carry):
        for m in range(3):
            wait_w(m, g)

        @pl.when(g < n_grp - 1)
        def _():
            for m in range(3):
                start_w(m, g + 1)

        @pl.when(g == n_grp - 1)
        def _():
            cp_x_tail.start()

        start_wo(g)
        for m in range(3):
            project_head(m, g)
        return carry

    lax.fori_loop(1, n_grp, prologue_body, 0)
    for c in cp_ffn:
        c.start()
    cp_x_tail.wait()
    pltpu.make_async_copy(wo_v, wo_v, sem_o).wait()

    def find_top2():
        pos = lax.broadcasted_iota(I32, (8, 128), 1) * 8 + lax.broadcasted_iota(I32, (8, 128), 0)
        vals = [r_v[i] for i in range(r_v.shape[0])]
        toks = [(pos + 1024 * i).astype(F32) for i in range(r_v.shape[0])]

        def largest(vs):
            m = functools.reduce(jnp.maximum, vs)
            return jnp.max(jnp.max(m, axis=0, keepdims=True), axis=1, keepdims=True)

        def first_with(vs, m):
            c = functools.reduce(jnp.minimum,
                                 [jnp.where(v == m, t, float(S)) for v, t in zip(vs, toks)])
            return jnp.min(jnp.min(c, axis=0, keepdims=True), axis=1, keepdims=True)

        m1 = largest(vals)
        j1 = first_with(vals, m1)
        vals = [jnp.where(t == j1, -jnp.inf, v) for v, t in zip(vals, toks)]
        m2 = largest(vals)
        j2 = first_with(vals, m2)
        for i, v in enumerate((m1, m2, j1, j2)):
            top_v[i] = jnp.broadcast_to(v, (8, 128))

    def head_cols(u):
        return slice(u * E, (u + 1) * E)

    def step(s, ffn_chunk=None, rank=False):
        row = lax.broadcasted_iota(I32, (L, L), 0)
        col = lax.broadcasted_iota(I32, (L, L), 1)
        mask = (row < M) | (row >= col)
        row0 = pl.multiple_of(s * seg, seg)
        new0 = pl.multiple_of(r0 + s * T, 8)
        ring_wr = pl.multiple_of(lax.rem(r0 + off + s * T, ring_rows), 8)
        ring_rd = pl.multiple_of(lax.rem(off + s * seg, ring_rows), seg)
        h = jnp.concatenate([mem_v[...], xn_v[pl.ds(new0, T), :]], axis=0).astype(BF16)

        def slot(g, u):
            return (g * G + u) % p_v.shape[0]

        def project(m, g):
            w = jnp.concatenate([w_vm[m][g * G + u] for u in range(G)], axis=1)
            y = _dot(h, _unpack(w))
            ring[m][g, pl.ds(ring_wr, T), :] = y[M:]
            for u in range(G):
                mem_rows[m][slot(g, u)] = y[0:M, head_cols(u)]

        def segment(m, g, u):
            return jnp.concatenate(
                [mem_rows[m][slot(g, u)], ring[m][g, pl.ds(ring_rd, seg), head_cols(u)]], axis=0)

        def probabilities(g):
            for u in range(G):
                sc = jnp.where(mask, _dot(segment(0, g, u), segment(1, g, u), _NT), -1e9 / scale)
                e = jnp.exp2((sc - jnp.max(sc, axis=-1, keepdims=True)) * (scale * _LOG2E))
                p_v[slot(g, u)] = e * _recip(jnp.sum(e, axis=-1, keepdims=True))

        def attend(g):
            for u in range(G):
                o_v[:, head_cols(g * G + u)] = _dot(p_v[slot(g, u)],
                                                    segment(2, g, u).astype(BF16))

        ys = [None, None]

        def project_out(g, half):
            w = wo_v[g * G * E // 2:(g + 1) * G * E // 2, half * HD:(half + 1) * HD]
            y = _dot(o_v[:, g * G * E:(g + 1) * G * E], _unpack(w))
            ys[half] = y if ys[half] is None else y + ys[half]

        ffn = {}

        def ffn_up(j):
            cols = pl.ds(pl.multiple_of(ffn_chunk * FC, 128), FC)
            rows = slice(j * 64, (j + 1) * 64)
            w = jnp.concatenate([wg_v[rows, cols], wu_v[rows, cols]], axis=1)
            t = _dot(xs_v[:, j * 128:(j + 1) * 128], _unpack(w))
            ffn["pre"] = t if j == 0 else t + ffn["pre"]

        def ffn_down(j):
            if "act" not in ffn:
                gate, up = ffn["pre"][:, :FC], ffn["pre"][:, FC:]
                ffn["act"] = gate * jax.nn.sigmoid(gate) * up
            kb, half = j % (FC // 128), j // (FC // 128)
            rows = pl.ds(pl.multiple_of(ffn_chunk * (FC // 2) + kb * 64, 64), 64)
            cols = slice(half * HD, (half + 1) * HD)
            yf_v[:, cols] = (_dot(ffn["act"][:, kb * 128:(kb + 1) * 128], _unpack(wd_v[rows, cols]))
                             + yf_v[:, cols])

        for g in range(n_grp):
            project(0, g)
            project(1, g)
            if ffn_chunk is None and g == n_grp - 3:
                normalise(pl.multiple_of(jnp.minimum(r0 + T + s * LN_STEP, S - LN_STEP), 8),
                          LN_STEP)
            if g > 0:
                attend(g - 1)
            if rank and g == 1:
                find_top2()
            project(2, g)
            probabilities(g)
        early = [(g, half) for half in range(2) for g in range(n_grp - 2)]
        late = [(g, half) for g in range(n_grp - 2, n_grp) for half in range(2)]
        n_up, n_down = D // 128, 2 * FC // 128
        for i, (g, half) in enumerate(early + late):
            if i == len(early):
                attend(n_grp - 1)
            project_out(g, half)
            if ffn_chunk is not None:
                if i < n_up:
                    ffn_up(i)
                if 0 <= i - (len(early) - 1) < n_down:
                    ffn_down(i - (len(early) - 1))

        y = jnp.concatenate(ys, axis=1)
        mem_v[...] = y[0:M]
        res = (x_v[pl.ds(row0, seg), :].astype(F32) + y[M:]) + xn_v[pl.ds(row0, seg), :]
        out_v[pl.ds(row0, seg), :] = res.astype(BF16)
        return out_copy(row0, seg, sem_out)

    def plain_steps(i, carry):
        for j in range(UNROLL):
            step(i * UNROLL + j, rank=(j == 0)).start()
        return carry

    lax.fori_loop(0, (n_seg - n_ffn) // UNROLL, plain_steps, 0)

    m1, m2, j1, j2 = (top_v[i] for i in range(4))
    t1 = jnp.clip(j1.astype(I32)[0, 0], 0, S - 1)
    t2 = jnp.clip(j2.astype(I32)[0, 0], 0, S - 1)

    first_row = lax.broadcasted_iota(I32, (8, D), 0) == 0
    xs_v[...] = jnp.where(first_row, xn_v[pl.ds(t1, 1), :], xn_v[pl.ds(t2, 1), :])
    yf_v[...] = jnp.zeros(yf_v.shape, F32)
    for c in cp_ffn:
        c.wait()

    def ffn_steps(i, carry):
        for j in range(UNROLL):
            copy = step(n_seg - n_ffn + i * UNROLL + j, i * UNROLL + j)
            if j < UNROLL - 1:
                copy.start()
            else:
                pl.when(i < n_ffn // UNROLL - 1)(copy.start)
        return carry

    lax.fori_loop(0, n_ffn // UNROLL, ffn_steps, 0)

    gate = jax.nn.sigmoid(jnp.where(lax.broadcasted_iota(I32, (8, 128), 0) == 0, m1, m2))
    yf = yf_v[...] * gate[:, 0:1]
    sent = out_v.at[pl.ds(0, S - seg), :]
    pltpu.make_async_copy(sent, sent, sem_out).wait()
    rows16 = lax.broadcasted_iota(I32, (16, D), 0)
    b1 = pl.multiple_of((t1 >> 4) << 4, 16)
    b2 = pl.multiple_of((t2 >> 4) << 4, 16)
    for b, t, i in ((b1, t1, 0), (b2, t2, 1)):
        blk = out_v[pl.ds(b, 16), :].astype(F32)
        out_v[pl.ds(b, 16), :] = jnp.where(rows16 == t - b, blk + yf[i:i + 1], blk).astype(BF16)

    last = out_copy(S - seg, seg, sem_out)
    last.start()
    resend = [(b1 < S - seg, out_copy(b1, 16, sem_p.at[0])),
              ((b2 < S - seg) & (b2 != b1), out_copy(b2, 16, sem_p.at[1]))]
    for cond, copy in resend:
        pl.when(cond)(copy.start)
    for cond, copy in resend:
        pl.when(cond)(copy.wait)
    last.wait()


@functools.partial(jax.jit, static_argnames=("A_seg_len",))
def pallas_parallel_sum__memory_aug_recurrent_mem_tr__moe_arch_mod__prompt_kernel(
    A_x, A_mem0, A_Wq, A_Wk, A_Wv, A_Wo, A_seg_len, B_x, B_w_r, B_w_gate, B_w_up, B_w_down,
):
    del B_x
    B, S, D = A_x.shape
    _, H, E = A_Wq.shape
    M = A_mem0.shape[1]
    F = B_w_gate.shape[1]
    seg = int(A_seg_len)
    L = M + seg
    n_seg, n_grp, n_ffn = S // seg, H // G, F // FC
    r0 = S - n_seg * T
    ring_rows, off = 576, 64
    assert B == 1 and S % seg == 0 and S % 1024 == 0 and E == 128 and F % FC == 0
    assert (r0 + off) % T == 0 and off % seg == 0 and ring_rows % T == 0 and ring_rows % seg == 0
    assert r0 + off <= ring_rows and r0 + T <= ring_rows and seg - T <= r0 // (n_seg - 1)
    assert r0 % LN_HEAD == 0 and r0 // LN_HEAD >= 3 and T <= seg and T <= LN_STEP
    assert r0 + T + (n_seg - n_ffn - UNROLL) * LN_STEP >= S
    assert n_ffn % UNROLL == 0 and n_seg % UNROLL == 0

    any_spec = pl.BlockSpec(memory_space=pl.ANY)
    out = pl.pallas_call(
        functools.partial(_kernel, seg=seg, r0=r0, off=off),
        out_shape=jax.ShapeDtypeStruct((S, D), A_x.dtype),
        in_specs=[any_spec] * 10,
        out_specs=any_spec,
        scratch_shapes=[
            pltpu.VMEM((S, D), BF16),
            pltpu.VMEM((S, D), F32),
            pltpu.VMEM((r0 // 2, D), I32),
            pltpu.VMEM((S, D), BF16),
            pltpu.VMEM((M, D), BF16),
            pltpu.VMEM((D // 128, 128), BF16),
            pltpu.VMEM((M, D), F32),
            pltpu.VMEM((L, H * E), F32),
            pltpu.VMEM((4 * G, L, L), F32),
            pltpu.VMEM((4 * G, M, E), F32),
            pltpu.VMEM((4 * G, M, E), F32),
            pltpu.VMEM((4 * G, M, E), F32),
            pltpu.VMEM((H, D // 2, E), I32),
            pltpu.VMEM((H, D // 2, E), I32),
            pltpu.VMEM((H, D // 2, E), I32),
            pltpu.VMEM((H * E // 2, D), I32),
            pltpu.VMEM((D // 2, F), I32),
            pltpu.VMEM((D // 2, F), I32),
            pltpu.VMEM((F // 2, D), I32),
            pltpu.VMEM((n_grp, ring_rows, G * E), F32),
            pltpu.VMEM((n_grp, ring_rows, G * E), F32),
            pltpu.VMEM((n_grp, ring_rows, G * E), F32),
            pltpu.VMEM((S // 1024, 8, 128), F32),
            pltpu.VMEM((8, D), F32),
            pltpu.VMEM((8, D), F32),
            pltpu.VMEM((4, 8, 128), F32),
            pltpu.SemaphoreType.DMA((2,)),
            pltpu.SemaphoreType.DMA((r0 // LN_HEAD + 1,)),
            pltpu.SemaphoreType.DMA((3, n_grp)),
            pltpu.SemaphoreType.DMA(()),
            pltpu.SemaphoreType.DMA((3,)),
            pltpu.SemaphoreType.DMA(()),
            pltpu.SemaphoreType.DMA((2,)),
        ],
        compiler_params=pltpu.CompilerParams(vmem_limit_bytes=120 * 1024 * 1024),
    )(
        A_x.reshape(S, D), A_mem0.reshape(M, D),
        A_Wq.reshape(D // 2, 2, H, E), A_Wk.reshape(D // 2, 2, H, E), A_Wv.reshape(D // 2, 2, H, E),
        A_Wo.reshape(H * E, D), B_w_r.reshape(D // 128, 128), B_w_gate, B_w_up, B_w_down,
    )
    return out.reshape(B, S, D)
```
